```python
import jax
import jax.numpy as jnp

def _softmax(x, axis=-1):
    return jax.nn.softmax(x, axis=axis)
def _gelu(x):
    return jax.nn.gelu(x, approximate=True)
def _silu(x):
    return jax.nn.silu(x)
def _sigmoid(x):
    return jax.nn.sigmoid(x)
def _layernorm(x, axis=-1, eps=1e-5):
    m = jnp.mean(x, axis=axis, keepdims=True)
    v = jnp.var(x, axis=axis, keepdims=True)
    return (x - m) / jnp.sqrt(v + eps)
def _scatter_add(tgt, idx, src, axis=0):
    return tgt.at[idx].add(src)
def _segment_sum(src, seg, n):
    return jax.ops.segment_sum(src, seg, n)
class _Rng:
    def __init__(self, key):
        self._k = key
    def _next(self):
        self._k, sub = jax.random.split(self._k)
        return sub
    def normal(self, shape):
        return jax.random.normal(self._next(), shape, dtype=jnp.bfloat16)
    def randint(self, lo, hi, shape):
        return jax.random.randint(self._next(), shape, lo, hi, dtype=jnp.int32)
    def uniform(self, shape, lo=0.0, hi=1.0):
        return jax.random.uniform(self._next(), shape, jnp.bfloat16, lo, hi)
    def permutation(self, n):
        return jax.random.permutation(self._next(), n)


kernel_name = 'gated_mix__compressed_kv_cla__sliding_local_dilated__prompt'

def setup_inputs():
    _rng = _Rng(jax.random.key(int.from_bytes(__import__("os").urandom(4), "little")))
    _w = (lambda a: (lambda t: t.astype(jnp.bfloat16) if jnp.issubdtype(t.dtype, jnp.floating) else t)(jnp.asarray(a)))
    def _A_setup():
        B, H, Sq, Sk, D, M = 1, 32, 2048, 2048, 128, 1024
        Dc = 4 * D
        return {
            "x": _w((lambda *s: _rng.normal(s) * 0.05)(B, Sq, M)),
            "c_kv": _w((lambda *s: _rng.normal(s) * 0.05)(B, Sk, Dc)),
            "w_q": _w((lambda *s: _rng.normal(s) * 0.05)(M, H, D) * (M ** -0.5)),
            "w_uk": _w((lambda *s: _rng.normal(s) * 0.05)(Dc, H, D) * (Dc ** -0.5)),
            "w_uv": _w((lambda *s: _rng.normal(s) * 0.05)(Dc, H, D) * (Dc ** -0.5)),
            "w_o": _w((lambda *s: _rng.normal(s) * 0.05)(H, D, M) * ((H * D) ** -0.5)),
        }
    _A_in = _A_setup()

    def _B_setup():
        B, S, D = 1, 2048, 1024
        return {
            "x": _w((lambda *s: _rng.normal(s) * 0.05)(B, S, D)),
            "wqkv": _w((lambda *s: _rng.normal(s) * 0.05)(D, 3 * D)),
            "wo": _w((lambda *s: _rng.normal(s) * 0.05)(D, D)),
        }
    _B_in = _B_setup()

    return {
        "A_x": _A_in["x"],
        "A_c_kv": _A_in["c_kv"],
        "A_w_q": _A_in["w_q"],
        "A_w_uk": _A_in["w_uk"],
        "A_w_uv": _A_in["w_uv"],
        "A_w_o": _A_in["w_o"],
        "B_x": _B_in["x"],
        "B_wqkv": _B_in["wqkv"],
        "B_wo": _B_in["wo"],
        "gate_w": _w((lambda *s: _rng.normal(s) * 0.05)(1024)),
    }

def reference(A_x, A_c_kv, A_w_q, A_w_uk, A_w_uv, A_w_o, B_x, B_wqkv, B_wo, gate_w):
    def _A_ref(x, c_kv, w_q, w_uk, w_uv, w_o):
        B, Sq, M = x.shape[0], x.shape[1], x.shape[2]
        Sk = c_kv.shape[1]
        H, D = w_q.shape[1], w_q.shape[2]
        q = jnp.einsum("bqm,mhd->bhqd", x, w_q)
        k = jnp.einsum("bkc,chd->bhkd", c_kv, w_uk)
        v = jnp.einsum("bkc,chd->bhkd", c_kv, w_uv)
        scores = jnp.einsum("bhqd,bhkd->bhqk", q, k) * (D ** -0.5)
        off = Sk - Sq
        qi = jnp.arange(Sq)[:, None]
        kj = jnp.arange(Sk)[None, :]
        cmask = kj <= (qi + off)
        scores = jnp.where(cmask[None, None], scores, -1e9)
        p = _softmax(scores, axis=-1)
        ctx = jnp.einsum("bhqk,bhkd->bhqd", p, v)
        return jnp.einsum("bhqd,hdm->bqm", ctx, w_o)

    def _B_ref(x, wqkv, wo):
        B, S, D = x.shape
        H = 32; Dh = D // H
        W, dil = 8, 2
        qkv = (lambda x, *d: x.transpose(*d))((x @ wqkv).reshape(B, S, 3, H, Dh), 2, 0, 3, 1, 4)
        q, k, v = qkv[0], qkv[1], qkv[2]
        scale = Dh ** -0.5
        pos = jnp.arange(S)
        off = jnp.arange(W) * dil
        idx = pos[:, None] - off[None, :]
        mask = idx >= 0
        idx_c = jnp.where(mask, idx, 0).reshape(-1)
        kg = k[:, :, idx_c, :].reshape(B, H, S, W, Dh)
        vg = v[:, :, idx_c, :].reshape(B, H, S, W, Dh)
        logits = jnp.einsum("bhsd,bhswd->bhsw", q, kg) * scale
        logits = jnp.where(mask[None, None, :, :], logits, -1e9)
        attn = _softmax(logits, axis=-1)
        o = jnp.einsum("bhsw,bhswd->bhsd", attn, vg)
        return (lambda x, *d: x.transpose(*d))(o, 0, 2, 1, 3).reshape(B, S, D) @ wo

    x = A_x
    g = _sigmoid((x * gate_w).sum(-1, keepdims=True))
    a = _A_ref(x, A_c_kv, A_w_q, A_w_uk, A_w_uv, A_w_o)
    b = _B_ref(x, B_wqkv, B_wo)
    return g * a + (1 - g) * b
```

```python
import functools
import jax
import jax.numpy as jnp
import numpy as np
import jax.experimental.pallas as pl
import jax.experimental.pallas.tpu as pltpu

S = 2048
M = 1024
H = 32
D = 128
DC = 512
DB = 1024
W = 8
DIL = 2
BQ = 512
RB = 256
F32 = jnp.float32
BF16 = jnp.bfloat16
LOG2E = 1.4426950408889634
DO_A = True
DO_B = True
DO_F = True
NT = (((1,), (1,)), ((), ()))


def _kernel(x_hbm, c_hbm, wq_hbm, wuk_hbm, wuv_hbm, wo_hbm, wqkv_hbm, wob_hbm, gate_ref,
            out_hbm,
            x_v, c_v, wq_v, wuk_v, wuv_v, wo_v, wqkv_v, wob_v, ctx_v, q_v, k_v, v_v,
            kb_v, vb_v, outs_v, sems, osems):
    def cp(src, dst, i):
        return pltpu.make_async_copy(src, dst, sems.at[i])

    cps = [cp(x_hbm, x_v, 0), cp(c_hbm, c_v, 1), cp(wq_hbm, wq_v, 2), cp(wuk_hbm, wuk_v, 3),
           cp(wuv_hbm, wuv_v, 4), cp(wqkv_hbm, wqkv_v, 5), cp(wob_hbm, wob_v, 6), cp(wo_hbm, wo_v, 7)]
    for c in cps:
        c.start()
    for i in range(5):
        cps[i].wait()

    qscale = (D ** -0.5) * LOG2E

    def head_body(h, carry):
        q = jnp.dot(x_v[...], wq_v[h], preferred_element_type=F32)
        q_v[...] = (q * qscale).astype(BF16)
        k_v[...] = jnp.dot(c_v[...], wuk_v[h], preferred_element_type=F32).astype(BF16)
        v_v[...] = jnp.dot(c_v[...], wuv_v[h], preferred_element_type=F32).astype(BF16)
        lane0 = pl.multiple_of(h * D, D)
        tri = (jax.lax.broadcasted_iota(jnp.int32, (128, 128), 1)
               <= jax.lax.broadcasted_iota(jnp.int32, (128, 128), 0))
        for qi in range(S // BQ):
            r0 = qi * BQ
            G = BQ // 128
            qb = q_v[r0:r0 + BQ, :]
            mt = None
            if qi > 0:
                sf = jax.lax.dot_general(qb, k_v[r0 * 0:r0, :], NT, preferred_element_type=F32)
                mt = functools.reduce(jnp.maximum, [sf[:, t * 128:(t + 1) * 128] for t in range(r0 // 128)])
            sd = []
            for j in range(G):
                sj = jax.lax.dot_general(qb[j * 128:], k_v[r0 + j * 128:r0 + (j + 1) * 128, :], NT,
                                         preferred_element_type=F32)
                top = jnp.where(tri, sj[:128], -1e30)
                sj = top if j == G - 1 else jnp.concatenate([top, sj[128:]], axis=0)
                sd.append(sj)
            mg = []
            for i in range(G):
                ts = [sd[j][(i - j) * 128:(i - j + 1) * 128] for j in range(i + 1)]
                if mt is not None:
                    ts.append(mt[i * 128:(i + 1) * 128])
                mg.append(functools.reduce(jnp.maximum, ts))
            m = jnp.max(jnp.concatenate(mg, axis=0), axis=1, keepdims=True)
            pds = [jnp.exp2(sd[j] - m[j * 128:]) for j in range(G)]
            lg = []
            lt = None
            if qi > 0:
                pf = jnp.exp2(sf - m)
                lt = functools.reduce(jnp.add, [pf[:, t * 128:(t + 1) * 128] for t in range(r0 // 128)])
                acc = jnp.dot(pf.astype(BF16), v_v[0:r0, :], preferred_element_type=F32)
            for i in range(G):
                ts = [pds[j][(i - j) * 128:(i - j + 1) * 128] for j in range(i + 1)]
                if lt is not None:
                    ts.append(lt[i * 128:(i + 1) * 128])
                lg.append(functools.reduce(jnp.add, ts))
            l = jnp.sum(jnp.concatenate(lg, axis=0), axis=1, keepdims=True)
            accs = [jnp.dot(pds[j].astype(BF16), v_v[r0 + j * 128:r0 + (j + 1) * 128, :],
                            preferred_element_type=F32) for j in range(G)]
            rl = 1.0 / l
            for i in range(G):
                ts = [accs[j][(i - j) * 128:(i - j + 1) * 128] for j in range(i + 1)]
                if qi > 0:
                    ts.append(acc[i * 128:(i + 1) * 128])
                o = functools.reduce(jnp.add, ts) * rl[i * 128:(i + 1) * 128]
                ctx_v[r0 + i * 128:r0 + (i + 1) * 128, pl.ds(lane0, D)] = o.astype(BF16)
        return carry

    if DO_A:
        jax.lax.fori_loop(0, H, head_body, 0)
    else:
        ctx_v[...] = jnp.zeros(ctx_v.shape, BF16)

    for i in range(5, 8):
        cps[i].wait()

    PAD = 16
    kb_v[0:PAD, :] = jnp.zeros((PAD, DB), F32)
    vb_v[0:PAD, :] = jnp.zeros((PAD, DB), F32)

    def kv_body(r, carry):
        r0 = pl.multiple_of(r * RB, RB)
        xb = x_v[pl.ds(r0, RB), :]
        kb_v[pl.ds(r0 + PAD, RB), :] = jnp.dot(xb, wqkv_v[:, DB:2 * DB], preferred_element_type=F32)
        vb_v[pl.ds(r0 + PAD, RB), :] = jnp.dot(xb, wqkv_v[:, 2 * DB:3 * DB], preferred_element_type=F32)
        return carry

    if DO_B:
        jax.lax.fori_loop(0, S // RB, kv_body, 0)

    bi = jax.lax.broadcasted_iota(jnp.int32, (128, 128), 0) // 32
    bj = jax.lax.broadcasted_iota(jnp.int32, (128, 128), 1) // 32
    ones_bd = jnp.where(bi == bj, 1.0, 0.0).astype(BF16)
    gw = gate_ref[...].astype(F32)
    bscale = (32 ** -0.5) * LOG2E

    def out_cp(r, slot):
        r0 = pl.multiple_of(r * RB, RB)
        return pltpu.make_async_copy(outs_v.at[slot], out_hbm.at[pl.ds(r0, RB), :], osems.at[slot])

    def fin_body(r, carry):
        r0 = pl.multiple_of(r * RB, RB)
        slot = r % 2
        xb = x_v[pl.ds(r0, RB), :]
        qb = jnp.dot(xb, wqkv_v[:, 0:DB], preferred_element_type=F32) * bscale
        kw = kb_v[pl.ds(r0, RB + PAD), :]
        vw = vb_v[pl.ds(r0, RB + PAD), :]
        row = r0 + jax.lax.broadcasted_iota(jnp.int32, (RB, 128), 0)
        ocols = []
        for lt in range(DB // 128):
            ql = qb[:, lt * 128:(lt + 1) * 128]
            logits = []
            for w in range(W):
                o = PAD - DIL * w
                kl = kw[o:o + RB, lt * 128:(lt + 1) * 128]
                lg = jnp.dot((ql * kl).astype(BF16), ones_bd, preferred_element_type=F32)
                if w > 0:
                    lg = jnp.where(row >= DIL * w, lg, -1e30)
                logits.append(lg)
            m = functools.reduce(jnp.maximum, logits)
            ps = [jnp.exp2(lg - m) for lg in logits]
            l = functools.reduce(jnp.add, ps)
            acc = None
            for w in range(W):
                o = PAD - DIL * w
                vl = vw[o:o + RB, lt * 128:(lt + 1) * 128]
                t = ps[w] * vl
                acc = t if acc is None else acc + t
            ocols.append((acc * (1.0 / l)).astype(BF16))
        ob = jnp.concatenate(ocols, axis=1)
        b = jnp.dot(ob, wob_v[...], preferred_element_type=F32)
        a = jnp.dot(ctx_v[pl.ds(r0, RB), :], wo_v[...], preferred_element_type=F32)
        g = jax.nn.sigmoid(jnp.sum(xb.astype(F32) * gw, axis=1, keepdims=True))
        res = g * a + (1.0 - g) * b

        @pl.when(r >= 2)
        def _():
            out_cp(r - 2, slot).wait()

        outs_v[slot] = res.astype(BF16)
        out_cp(r, slot).start()
        return carry

    nb = S // RB
    jax.lax.fori_loop(0, nb, fin_body, 0)
    out_cp(nb - 2, (nb - 2) % 2).wait()
    out_cp(nb - 1, (nb - 1) % 2).wait()


@jax.jit
def pallas_gated_mix__compressed_kv_cla__sliding_local_dilated__prompt_kernel(
    A_x, A_c_kv, A_w_q, A_w_uk, A_w_uv, A_w_o, B_x, B_wqkv, B_wo, gate_w):
    x = A_x.reshape(S, M)
    c = A_c_kv.reshape(S, DC)
    wq = A_w_q.transpose(1, 0, 2)
    wuk = A_w_uk.transpose(1, 0, 2)
    wuv = A_w_uv.transpose(1, 0, 2)
    wo = A_w_o.reshape(H * D, M)
    gw = gate_w.reshape(1, M)
    anyspec = pl.BlockSpec(memory_space=pl.ANY)
    out = pl.pallas_call(
        _kernel,
        grid=(1,),
        in_specs=[anyspec] * 8 + [pl.BlockSpec((1, M), lambda i: (0, 0))],
        out_specs=anyspec,
        out_shape=jax.ShapeDtypeStruct((S, M), BF16),
        scratch_shapes=[
            pltpu.VMEM((S, M), BF16), pltpu.VMEM((S, DC), BF16),
            pltpu.VMEM((H, M, D), BF16), pltpu.VMEM((H, DC, D), BF16), pltpu.VMEM((H, DC, D), BF16),
            pltpu.VMEM((H * D, M), BF16), pltpu.VMEM((M, 3 * DB), BF16), pltpu.VMEM((DB, DB), BF16),
            pltpu.VMEM((S, H * D), BF16),
            pltpu.VMEM((S, D), BF16), pltpu.VMEM((S, D), BF16), pltpu.VMEM((S, D), BF16),
            pltpu.VMEM((S + 16, DB), F32), pltpu.VMEM((S + 16, DB), F32),
            pltpu.VMEM((2, RB, M), BF16),
            pltpu.SemaphoreType.DMA((8,)), pltpu.SemaphoreType.DMA((2,)),
        ],
        compiler_params=pltpu.CompilerParams(
            dimension_semantics=("arbitrary",), vmem_limit_bytes=110 * 1024 * 1024),
    )(x, c, wq, wuk, wuv, wo, B_wqkv, B_wo, gw)
    return out.reshape(1, S, M)
```

```python
import functools
import jax
import jax.numpy as jnp
import jax.experimental.pallas as pl
import jax.experimental.pallas.tpu as pltpu

S = 2048
M = 1024
H = 32
D = 128
DC = 512
DB = 1024
W = 8
DIL = 2
BQ = 512
RB = 256
PAD = 16
NT1 = 16
NSLOT = 3
F32 = jnp.float32
BF16 = jnp.bfloat16
U32 = jnp.uint32
LOG2E = 1.4426950408889634
NEG = -1e30
NT = (((1,), (1,)), ((), ()))
FLAGS = {}
ORDER = lambda n: range(n - 1, -1, -1)
KCH = 512


def _kernel(x_hbm, c_hbm, wq_hbm, wuk_hbm, wuv_hbm, wo_hbm, wqkv_hbm, wob_hbm, gate_ref,
            out_hbm,
            x_v, c_v, wq_v, wuk_v, wuv_v, wo_v, wqb_v, wkvb_v, wob_v, ctx_v, q_v, k_v, v_v,
            kvb_v, rq_v, ruk_v, ruv_v, outs_v, xsem, rsem, wsem, osems):
    nrb = S // RB
    RQ = M * H // NT1
    RU = DC * H // NT1

    def x_cp(r):
        r0 = pl.multiple_of(r * RB, RB)
        return pltpu.make_async_copy(x_hbm.at[pl.ds(r0, RB), :], x_v.at[pl.ds(r0, RB), :], xsem.at[r])

    def raw_cps(t, slot):
        return [
            pltpu.make_async_copy(wq_hbm.at[pl.ds(pl.multiple_of(t * RQ, RQ), RQ), :], rq_v.at[slot], rsem.at[0, slot]),
            pltpu.make_async_copy(wuk_hbm.at[pl.ds(pl.multiple_of(t * RU, RU), RU), :], ruk_v.at[slot], rsem.at[1, slot]),
            pltpu.make_async_copy(wuv_hbm.at[pl.ds(pl.multiple_of(t * RU, RU), RU), :], ruv_v.at[slot], rsem.at[2, slot]),
        ]

    wk_cp = pltpu.make_async_copy(wqkv_hbm.at[:, pl.ds(DB, DB)], wkvb_v.at[0], wsem.at[0])
    wv_cp = pltpu.make_async_copy(wqkv_hbm.at[:, pl.ds(2 * DB, DB)], wkvb_v.at[1], wsem.at[1])
    wqb_cp = pltpu.make_async_copy(wqkv_hbm.at[:, pl.ds(0, DB)], wqb_v, wsem.at[2])
    wob_cp = pltpu.make_async_copy(wob_hbm, wob_v, wsem.at[3])
    wo_cp = pltpu.make_async_copy(wo_hbm, wo_v, wsem.at[4])
    c_cp = pltpu.make_async_copy(c_hbm, c_v, wsem.at[5])

    x_cp(0).start()
    wk_cp.start()
    for c in raw_cps(0, 0):
        c.start()
    x_cp(1).start()
    for c in raw_cps(1, 1):
        c.start()

    kvb_v[0, 0:PAD, :] = jnp.zeros((PAD, DB), F32)
    kvb_v[1, 0:PAD, :] = jnp.zeros((PAD, DB), F32)
    wk_cp.wait()

    rq_u = rq_v.bitcast(U32)
    ruk_u = ruk_v.bitcast(U32)
    ruv_u = ruv_v.bitcast(U32)

    def relayout(src_u, slot, dst, row0, nrows):
        for j in range(H // 2):
            u = src_u[slot, pl.ds(j, nrows, stride=H // 2), :]
            lo = pltpu.bitcast(u << 16, F32).astype(BF16)
            hi = pltpu.bitcast(u & jnp.uint32(0xFFFF0000), F32).astype(BF16)
            dst[2 * j, pl.ds(row0, nrows), :] = lo
            dst[2 * j + 1, pl.ds(row0, nrows), :] = hi

    def p1_body(t, carry):
        mat = t // nrb
        r = t % nrb
        slot = t % NSLOT

        @pl.when(t + 2 < NT1)
        def _():
            for c in raw_cps(t + 2, (t + 2) % NSLOT):
                c.start()

        @pl.when(t + 2 < nrb)
        def _():
            x_cp(t + 2).start()

        @pl.when(t == 1)
        def _():
            wv_cp.start()

        @pl.when(t == 6)
        def _():
            c_cp.start()

        @pl.when(t == 9)
        def _():
            wqb_cp.start()
            wob_cp.start()

        @pl.when(t < nrb)
        def _():
            x_cp(t).wait()

        @pl.when(t == nrb)
        def _():
            wv_cp.wait()

        for c in raw_cps(t, slot):
            c.wait()
        r0 = pl.multiple_of(r * RB, RB)
        xb = x_v[pl.ds(r0, RB), :]
        kvb_v[mat, pl.ds(r0 + PAD, RB), :] = jnp.dot(xb, wkvb_v[mat], preferred_element_type=F32)
        relayout(rq_u, slot, wq_v, pl.multiple_of(t * (M // NT1), M // NT1), M // NT1)
        relayout(ruk_u, slot, wuk_v, pl.multiple_of(t * (DC // NT1), DC // NT1), DC // NT1)
        relayout(ruv_u, slot, wuv_v, pl.multiple_of(t * (DC // NT1), DC // NT1), DC // NT1)
        return carry

    jax.lax.fori_loop(0, NT1, p1_body, 0)
    wo_cp.start()
    c_cp.wait()

    qscale = (D ** -0.5) * LOG2E

    def head_body(h, carry):
        q = jnp.dot(x_v[...], wq_v[h], preferred_element_type=F32)
        q_v[...] = (q * qscale).astype(BF16)
        k_v[...] = jnp.dot(c_v[...], wuk_v[h], preferred_element_type=F32).astype(BF16)
        v_v[...] = jnp.dot(c_v[...], wuv_v[h], preferred_element_type=F32).astype(BF16)
        lane0 = pl.multiple_of(h * D, D)
        tri = (jax.lax.broadcasted_iota(jnp.int32, (128, 128), 1)
               <= jax.lax.broadcasted_iota(jnp.int32, (128, 128), 0))
        for qi in ORDER(S // BQ):
            r0 = qi * BQ
            G = BQ // 128
            qb = q_v[r0:r0 + BQ, :]
            mt = None
            if qi > 0:
                sf = jax.lax.dot_general(qb, k_v[0:r0, :], NT, preferred_element_type=F32)
                mt = functools.reduce(jnp.maximum, [sf[:, t * 128:(t + 1) * 128] for t in range(r0 // 128)])
            sd = []
            for j in range(G):
                sj = jax.lax.dot_general(qb[j * 128:], k_v[r0 + j * 128:r0 + (j + 1) * 128, :], NT,
                                         preferred_element_type=F32)
                top = jnp.where(tri, sj[:128], NEG)
                sd.append(top if j == G - 1 else jnp.concatenate([top, sj[128:]], axis=0))
            mg = []
            for i in range(G):
                ts = [sd[j][(i - j) * 128:(i - j + 1) * 128] for j in range(i + 1)]
                if mt is not None:
                    ts.append(mt[i * 128:(i + 1) * 128])
                mg.append(functools.reduce(jnp.maximum, ts))
            m = jnp.max(jnp.concatenate(mg, axis=0), axis=1, keepdims=True)
            pds = [jnp.exp2(sd[j] - m[j * 128:]) for j in range(G)]
            lg = []
            lt = None
            if qi > 0:
                pf = jnp.exp2(sf - m)
                lt = functools.reduce(jnp.add, [pf[:, t * 128:(t + 1) * 128] for t in range(r0 // 128)])
                acc = jnp.dot(pf.astype(BF16), v_v[0:r0, :], preferred_element_type=F32)
            for i in range(G):
                ts = [pds[j][(i - j) * 128:(i - j + 1) * 128] for j in range(i + 1)]
                if lt is not None:
                    ts.append(lt[i * 128:(i + 1) * 128])
                lg.append(functools.reduce(jnp.add, ts))
            l = jnp.sum(jnp.concatenate(lg, axis=0), axis=1, keepdims=True)
            accs = [jnp.dot(pds[j].astype(BF16), v_v[r0 + j * 128:r0 + (j + 1) * 128, :],
                            preferred_element_type=F32) for j in range(G)]
            rl = 1.0 / l
            for i in range(G):
                ts = [accs[j][(i - j) * 128:(i - j + 1) * 128] for j in range(i + 1)]
                if qi > 0:
                    ts.append(acc[i * 128:(i + 1) * 128])
                o = functools.reduce(jnp.add, ts) * rl[i * 128:(i + 1) * 128]
                ctx_v[r0 + i * 128:r0 + (i + 1) * 128, pl.ds(lane0, D)] = o.astype(BF16)
        return carry

    jax.lax.fori_loop(0, H, head_body, 0)
    wqb_cp.wait()
    wob_cp.wait()
    wo_cp.wait()

    bi = jax.lax.broadcasted_iota(jnp.int32, (128, 128), 0) // 32
    bj = jax.lax.broadcasted_iota(jnp.int32, (128, 128), 1) // 32
    ones_bd = jnp.where(bi == bj, 1.0, 0.0).astype(BF16)
    gw = gate_ref[...].astype(F32)
    bscale = (32 ** -0.5) * LOG2E

    def out_cp(r, slot):
        r0 = pl.multiple_of(r * RB, RB)
        return pltpu.make_async_copy(outs_v.at[slot], out_hbm.at[pl.ds(r0, RB), :], osems.at[slot])

    def fin_body(r, carry):
        r0 = pl.multiple_of(r * RB, RB)
        slot = r % 2
        xb = x_v[pl.ds(r0, RB), :]
        qb = jnp.dot(xb, wqb_v[...], preferred_element_type=F32) * bscale
        row = r0 + jax.lax.broadcasted_iota(jnp.int32, (PAD, 128), 0)
        a = None
        b = None
        for lt in range(DB // 128):
            cs = slice(lt * 128, (lt + 1) * 128)
            kw = kvb_v[0, pl.ds(r0, RB + PAD), cs]
            vw = kvb_v[1, pl.ds(r0, RB + PAD), cs]
            ql = qb[:, cs]
            logits = []
            for w in range(W):
                o = PAD - DIL * w
                lg = jnp.dot((ql * kw[o:o + RB]).astype(BF16), ones_bd, preferred_element_type=F32)
                if w > 0:
                    lg = jnp.concatenate([jnp.where(row >= DIL * w, lg[:PAD], NEG), lg[PAD:]], axis=0)
                logits.append(lg)
            for kc in range(lt * (H * D // 8) // KCH, (lt + 1) * (H * D // 8) // KCH):
                ks = slice(kc * KCH, (kc + 1) * KCH)
                at = jnp.dot(ctx_v[pl.ds(r0, RB), ks], wo_v[ks, :], preferred_element_type=F32)
                a = at if a is None else a + at
            m = functools.reduce(jnp.maximum, logits)
            ps = [jnp.exp2(lg - m) for lg in logits]
            l = functools.reduce(jnp.add, ps)
            acc = None
            for w in range(W):
                o = PAD - DIL * w
                t = ps[w] * vw[o:o + RB]
                acc = t if acc is None else acc + t
            ol = (acc * (1.0 / l)).astype(BF16)
            bt = jnp.dot(ol, wob_v[cs, :], preferred_element_type=F32)
            b = bt if b is None else b + bt
        g = jax.nn.sigmoid(jnp.sum(xb.astype(F32) * gw, axis=1, keepdims=True))
        res = g * a + (1.0 - g) * b

        @pl.when(r >= 2)
        def _():
            out_cp(r - 2, slot).wait()

        outs_v[slot] = res.astype(BF16)
        out_cp(r, slot).start()
        return carry

    jax.lax.fori_loop(0, nrb, fin_body, 0)
    out_cp(nrb - 2, (nrb - 2) % 2).wait()
    out_cp(nrb - 1, (nrb - 1) % 2).wait()


@jax.jit
def pallas_gated_mix__compressed_kv_cla__sliding_local_dilated__prompt_kernel(
    A_x, A_c_kv, A_w_q, A_w_uk, A_w_uv, A_w_o, B_x, B_wqkv, B_wo, gate_w):
    x = A_x.reshape(S, M)
    c = A_c_kv.reshape(S, DC)
    wq = A_w_q.reshape(M * H, D)
    wuk = A_w_uk.reshape(DC * H, D)
    wuv = A_w_uv.reshape(DC * H, D)
    wo = A_w_o.reshape(H * D, M)
    gw = gate_w.reshape(1, M)
    anyspec = pl.BlockSpec(memory_space=pl.ANY)
    out = pl.pallas_call(
        _kernel,
        grid=(1,),
        in_specs=[anyspec] * 8 + [pl.BlockSpec((1, M), lambda i: (0, 0))],
        out_specs=anyspec,
        out_shape=jax.ShapeDtypeStruct((S, M), BF16),
        scratch_shapes=[
            pltpu.VMEM((S, M), BF16), pltpu.VMEM((S, DC), BF16),
            pltpu.VMEM((H, M, D), BF16), pltpu.VMEM((H, DC, D), BF16), pltpu.VMEM((H, DC, D), BF16),
            pltpu.VMEM((H * D, M), BF16), pltpu.VMEM((M, DB), BF16), pltpu.VMEM((2, M, DB), BF16),
            pltpu.VMEM((DB, DB), BF16),
            pltpu.VMEM((S, H * D), BF16),
            pltpu.VMEM((S, D), BF16), pltpu.VMEM((S, D), BF16), pltpu.VMEM((S, D), BF16),
            pltpu.VMEM((2, S + PAD, DB), F32),
            pltpu.VMEM((NSLOT, M * H // NT1, D), BF16), pltpu.VMEM((NSLOT, DC * H // NT1, D), BF16),
            pltpu.VMEM((NSLOT, DC * H // NT1, D), BF16),
            pltpu.VMEM((2, RB, M), BF16),
            pltpu.SemaphoreType.DMA((S // RB,)), pltpu.SemaphoreType.DMA((3, NSLOT)),
            pltpu.SemaphoreType.DMA((6,)), pltpu.SemaphoreType.DMA((2,)),
        ],
        compiler_params=pltpu.CompilerParams(
            dimension_semantics=("arbitrary",), flags=FLAGS, vmem_limit_bytes=110 * 1024 * 1024),
    )(x, c, wq, wuk, wuv, wo, B_wqkv, B_wo, gw)
    return out.reshape(1, S, M)
```

```python
import functools
import jax
import jax.numpy as jnp
import jax.experimental.pallas as pl
import jax.experimental.pallas.tpu as pltpu

S = 2048
M = 1024
H = 32
D = 128
DC = 512
DB = 1024
W = 8
DIL = 2
BQ = 512
RB = 256
PAD = 16
NT1 = 16
NSLOT = 3
F32 = jnp.float32
BF16 = jnp.bfloat16
U32 = jnp.uint32
LOG2E = 1.4426950408889634
NEG = -1e30
NT = (((1,), (1,)), ((), ()))
FLAGS = {}
ORDER = lambda n: range(n - 1, -1, -1)
P1SPLIT = 4
FINSPLIT = 4
KCH = 512


def _pk(v):
    return pltpu.bitcast(v.astype(BF16), U32)


def _up(u):
    return pltpu.bitcast(u, BF16)


def _swap_lane_tiles(u):
    lane = jax.lax.broadcasted_iota(jnp.int32, (u.shape[0], 128), 1)
    t = [u[:, i * 128:(i + 1) * 128] for i in range(8)]
    for b in range(3):
        s = 4 << b
        lo = (lane & s) == 0
        n = list(t)
        for i in range(8):
            if not (i >> b) & 1:
                A, B = t[i], t[i | (1 << b)]
                n[i] = jnp.where(lo, A, pltpu.roll(B, s, 1))
                n[i | (1 << b)] = jnp.where(lo, pltpu.roll(A, 128 - s, 1), B)
        t = n
    return jnp.concatenate(t, axis=1)


def _kernel(x_hbm, c_hbm, wq_hbm, wuk_hbm, wuv_hbm, wo_hbm, wqkv_hbm, wob_hbm, gate_ref,
            out_hbm,
            xu, cu, wq_u, wuk_u, wuv_u, wo_u, wqb_u, wkvb_u, wob_u, ctx_u, q_u, k_u, v_u,
            kvb_v, rq_v, ruk_v, ruv_v, rx_v, rc_v, rkv_v, jo_v, jq_v, jb_v, outs_v,
            rsem, wsem, jsem, osems):
    nrb = S // RB
    RQ = M * H // NT1
    RU = DC * H // NT1
    RC = S // NT1

    def x_cp(r, slot):
        return pltpu.make_async_copy(x_hbm.at[pl.ds(pl.multiple_of(r * RB, RB), RB), :], rx_v.at[slot], rsem.at[4, slot])

    def raw_cps(t, slot):
        return [
            pltpu.make_async_copy(wq_hbm.at[pl.ds(pl.multiple_of(t * RQ, RQ), RQ), :], rq_v.at[slot], rsem.at[0, slot]),
            pltpu.make_async_copy(wuk_hbm.at[pl.ds(pl.multiple_of(t * RU, RU), RU), :], ruk_v.at[slot], rsem.at[1, slot]),
            pltpu.make_async_copy(wuv_hbm.at[pl.ds(pl.multiple_of(t * RU, RU), RU), :], ruv_v.at[slot], rsem.at[2, slot]),
            pltpu.make_async_copy(c_hbm.at[pl.ds(pl.multiple_of(t * RC, RC), RC), :], rc_v.at[slot], rsem.at[3, slot]),
        ]

    def job_cps(h, slot):
        return [
            pltpu.make_async_copy(wo_hbm.at[pl.ds(pl.multiple_of(h * D, D), D), :], jo_v.at[slot], jsem.at[0, slot]),
            pltpu.make_async_copy(wqkv_hbm.at[pl.ds(pl.multiple_of(h * 32, 32), 32), pl.ds(0, DB)], jq_v.at[slot], jsem.at[1, slot]),
            pltpu.make_async_copy(wob_hbm.at[pl.ds(pl.multiple_of(h * 32, 32), 32), :], jb_v.at[slot], jsem.at[2, slot]),
        ]

    wk_cp = pltpu.make_async_copy(wqkv_hbm.at[:, pl.ds(DB, DB)], rkv_v.at[0], wsem.at[0])
    wv_cp = pltpu.make_async_copy(wqkv_hbm.at[:, pl.ds(2 * DB, DB)], rkv_v.at[1], wsem.at[1])

    wk_cp.start()
    x_cp(0, 0).start()
    for c in raw_cps(0, 0):
        c.start()
    x_cp(1, 1).start()
    for c in raw_cps(1, 1):
        c.start()

    kvb_v[0, 0:PAD, :] = jnp.zeros((PAD, DB), F32)
    kvb_v[1, 0:PAD, :] = jnp.zeros((PAD, DB), F32)
    wk_cp.wait()
    for i in range(4):
        wkvb_u[0, i * 128:(i + 1) * 128, :] = _swap_lane_tiles(_pk(rkv_v[0, i * 256:(i + 1) * 256, :]))

    rq_u = rq_v.bitcast(U32)
    ruk_u = ruk_v.bitcast(U32)
    ruv_u = ruv_v.bitcast(U32)

    def relayout(src_u, slot, dst, row0, nrows, js):
        for j in js:
            u = src_u[slot, pl.ds(j, nrows, stride=H // 2), :]
            lo = pltpu.bitcast(u << 16, F32)
            hi = pltpu.bitcast(u & jnp.uint32(0xFFFF0000), F32)
            dst[2 * j, pl.ds(row0, nrows // 2), :] = _pk(lo)
            dst[2 * j + 1, pl.ds(row0, nrows // 2), :] = _pk(hi)

    def p1_body(t, carry):
        mat = t // nrb
        r = t % nrb
        slot = t % NSLOT

        @pl.when(t + 2 < NT1)
        def _():
            for c in raw_cps(t + 2, (t + 2) % NSLOT):
                c.start()

        @pl.when(t + 2 < nrb)
        def _():
            x_cp(t + 2, (t + 2) % NSLOT).start()

        @pl.when(t == 1)
        def _():
            wv_cp.start()

        @pl.when(t == NT1 - 2)
        def _():
            for c in job_cps(0, 0):
                c.start()

        @pl.when(t < nrb)
        def _():
            x_cp(t, slot).wait()
            xu[pl.ds(pl.multiple_of(t * (RB // 2), RB // 2), RB // 2), :] = _pk(rx_v[slot])

        @pl.when(t == nrb)
        def _():
            wv_cp.wait()
            for i in range(4):
                wkvb_u[1, i * 128:(i + 1) * 128, :] = _swap_lane_tiles(_pk(rkv_v[1, i * 256:(i + 1) * 256, :]))

        for c in raw_cps(t, slot):
            c.wait()
        r0 = pl.multiple_of(r * RB, RB)
        hq = pl.multiple_of(t * (M // NT1 // 2), M // NT1 // 2)
        hu = pl.multiple_of(t * (DC // NT1 // 2), DC // NT1 // 2)
        xb = _up(xu[pl.ds(pl.multiple_of(r * (RB // 2), RB // 2), RB // 2), :])
        NP = P1SPLIT
        for p in range(NP):
            cs = slice(p * (DB // NP), (p + 1) * (DB // NP))
            kvb_v[mat, pl.ds(r0 + PAD, RB), cs] = jnp.dot(xb, _up(wkvb_u[mat, :, cs]), preferred_element_type=F32)
            js = range(p * (16 // NP), (p + 1) * (16 // NP))
            relayout(rq_u, slot, wq_u, hq, M // NT1, js)
            relayout(ruk_u, slot, wuk_u, hu, DC // NT1, js)
            relayout(ruv_u, slot, wuv_u, hu, DC // NT1, js)
        cu[pl.ds(pl.multiple_of(t * (RC // 2), RC // 2), RC // 2), :] = _pk(rc_v[slot])
        return carry

    jax.lax.fori_loop(0, NT1, p1_body, 0)

    qscale = (D ** -0.5) * LOG2E

    def head_body(h, carry):
        js = h % 2

        @pl.when(h + 1 < H)
        def _():
            for c in job_cps(h + 1, 1 - js):
                c.start()

        for c in job_cps(h, js):
            c.wait()
        q = jnp.dot(_up(xu[...]), _up(wq_u[h]), preferred_element_type=F32)
        q_u[...] = _pk(q * qscale)
        cb = _up(cu[...])
        k_u[...] = _pk(jnp.dot(cb, _up(wuk_u[h]), preferred_element_type=F32))
        v_u[...] = _pk(jnp.dot(cb, _up(wuv_u[h]), preferred_element_type=F32))
        wo_u[pl.ds(pl.multiple_of(h * (D // 2), D // 2), D // 2), :] = _pk(jo_v[js])
        wqb_u[pl.ds(pl.multiple_of(h * 16, 16), 16), :] = _swap_lane_tiles(_pk(jq_v[js]))
        wob_u[pl.ds(pl.multiple_of(h * 16, 16), 16), :] = _pk(jb_v[js])
        lane0 = pl.multiple_of(h * D, D)
        tri = (jax.lax.broadcasted_iota(jnp.int32, (128, 128), 1)
               <= jax.lax.broadcasted_iota(jnp.int32, (128, 128), 0))
        for qi in ORDER(S // BQ):
            r0 = qi * BQ
            G = BQ // 128
            qb = _up(q_u[r0 // 2:(r0 + BQ) // 2, :])
            mt = None
            if qi > 0:
                sf = jax.lax.dot_general(qb, _up(k_u[0:r0 // 2, :]), NT, preferred_element_type=F32)
                mt = functools.reduce(jnp.maximum, [sf[:, t * 128:(t + 1) * 128] for t in range(r0 // 128)])
            sd = []
            for j in range(G):
                kj = _up(k_u[(r0 + j * 128) // 2:(r0 + (j + 1) * 128) // 2, :])
                sj = jax.lax.dot_general(qb[j * 128:], kj, NT, preferred_element_type=F32)
                top = jnp.where(tri, sj[:128], NEG)
                sd.append(top if j == G - 1 else jnp.concatenate([top, sj[128:]], axis=0))
            mg = []
            for i in range(G):
                ts = [sd[j][(i - j) * 128:(i - j + 1) * 128] for j in range(i + 1)]
                if mt is not None:
                    ts.append(mt[i * 128:(i + 1) * 128])
                mg.append(functools.reduce(jnp.maximum, ts))
            m = jnp.max(jnp.concatenate(mg, axis=0), axis=1, keepdims=True)
            pds = [jnp.exp2(sd[j] - m[j * 128:]) for j in range(G)]
            lg = []
            lt = None
            if qi > 0:
                pf = jnp.exp2(sf - m)
                lt = functools.reduce(jnp.add, [pf[:, t * 128:(t + 1) * 128] for t in range(r0 // 128)])
                acc = jnp.dot(pf.astype(BF16), _up(v_u[0:r0 // 2, :]), preferred_element_type=F32)
            for i in range(G):
                ts = [pds[j][(i - j) * 128:(i - j + 1) * 128] for j in range(i + 1)]
                if lt is not None:
                    ts.append(lt[i * 128:(i + 1) * 128])
                lg.append(functools.reduce(jnp.add, ts))
            l = jnp.sum(jnp.concatenate(lg, axis=0), axis=1, keepdims=True)
            accs = [jnp.dot(pds[j].astype(BF16), _up(v_u[(r0 + j * 128) // 2:(r0 + (j + 1) * 128) // 2, :]),
                            preferred_element_type=F32) for j in range(G)]
            rl = 1.0 / l
            for i in range(G):
                ts = [accs[j][(i - j) * 128:(i - j + 1) * 128] for j in range(i + 1)]
                if qi > 0:
                    ts.append(acc[i * 128:(i + 1) * 128])
                o = functools.reduce(jnp.add, ts) * rl[i * 128:(i + 1) * 128]
                ctx_u[(r0 + i * 128) // 2:(r0 + (i + 1) * 128) // 2, pl.ds(lane0, D)] = _pk(o)
        return carry

    jax.lax.fori_loop(0, H, head_body, 0)

    gw = gate_ref[...].astype(F32)
    bscale = (32 ** -0.5) * LOG2E

    def out_cp(r, slot):
        r0 = pl.multiple_of(r * RB, RB)
        return pltpu.make_async_copy(outs_v.at[slot], out_hbm.at[pl.ds(r0, RB), :], osems.at[slot])

    def fin_body(r, carry):
        r0 = pl.multiple_of(r * RB, RB)
        hr = pl.multiple_of(r * (RB // 2), RB // 2)
        slot = r % 2
        xb = _up(xu[pl.ds(hr, RB // 2), :])
        qb = jnp.dot(xb, _up(wqb_u[...]), preferred_element_type=F32) * bscale
        NS = FINSPLIT
        RS = RB // NS
        lane = jax.lax.broadcasted_iota(jnp.int32, (RS, 128), 1)
        odd1 = (lane & 1) == 1
        odd2 = (lane & 2) == 2
        a = None
        outs = []
        for sc in range(NS):
            s0 = sc * RS
            kw = kvb_v[0, pl.ds(r0 + s0, RS + PAD), :]
            vw = kvb_v[1, pl.ds(r0 + s0, RS + PAD), :]
            logits = []
            for w in range(W):
                o = PAD - DIL * w
                pr = qb[s0:s0 + RS] * kw[o:o + RS]
                lg = functools.reduce(jnp.add, [pr[:, t * 128:(t + 1) * 128] for t in range(8)])
                lg = lg + jnp.where(odd1, pltpu.roll(lg, 1, 1), pltpu.roll(lg, 127, 1))
                lg = lg + jnp.where(odd2, pltpu.roll(lg, 2, 1), pltpu.roll(lg, 126, 1))
                if w > 0 and s0 < PAD:
                    row = r0 + jax.lax.broadcasted_iota(jnp.int32, (PAD, 128), 0)
                    top = jnp.where(row >= DIL * w, lg[:PAD], NEG)
                    lg = top if RS == PAD else jnp.concatenate([top, lg[PAD:]], axis=0)
                logits.append(lg)
            for kc in range(sc * (8 // NS) * (512 // KCH), (sc + 1) * (8 // NS) * (512 // KCH)):
                ks = slice(kc * KCH, (kc + 1) * KCH)
                hs = slice(kc * KCH // 2, (kc + 1) * KCH // 2)
                at = jnp.dot(_up(ctx_u[pl.ds(hr, RB // 2), ks]), _up(wo_u[hs, :]), preferred_element_type=F32)
                a = at if a is None else a + at
            m = functools.reduce(jnp.maximum, logits)
            ps = [jnp.exp2(lg - m) for lg in logits]
            rl = 1.0 / functools.reduce(jnp.add, ps)
            ps = [p * rl for p in ps]
            cols = []
            for t in range(8):
                cs = slice(t * 128, (t + 1) * 128)
                acc = None
                for w in range(W):
                    o = PAD - DIL * w
                    tt = ps[w] * vw[o:o + RS, cs]
                    acc = tt if acc is None else acc + tt
                cols.append(acc)
            outs.append(_swap_lane_tiles(_pk(jnp.concatenate(cols, axis=1))))
        ob = _up(jnp.concatenate(outs, axis=0))
        b = jnp.dot(ob, _up(wob_u[...]), preferred_element_type=F32)
        g = jax.nn.sigmoid(jnp.sum(xb.astype(F32) * gw, axis=1, keepdims=True))
        res = g * a + (1.0 - g) * b

        @pl.when(r >= 2)
        def _():
            out_cp(r - 2, slot).wait()

        outs_v[slot] = res.astype(BF16)
        out_cp(r, slot).start()
        return carry

    jax.lax.fori_loop(0, nrb, fin_body, 0)
    out_cp(nrb - 2, (nrb - 2) % 2).wait()
    out_cp(nrb - 1, (nrb - 1) % 2).wait()


@jax.jit
def pallas_gated_mix__compressed_kv_cla__sliding_local_dilated__prompt_kernel(
    A_x, A_c_kv, A_w_q, A_w_uk, A_w_uv, A_w_o, B_x, B_wqkv, B_wo, gate_w):
    x = A_x.reshape(S, M)
    c = A_c_kv.reshape(S, DC)
    wq = A_w_q.reshape(M * H, D)
    wuk = A_w_uk.reshape(DC * H, D)
    wuv = A_w_uv.reshape(DC * H, D)
    wo = A_w_o.reshape(H * D, M)
    gw = gate_w.reshape(1, M)
    anyspec = pl.BlockSpec(memory_space=pl.ANY)
    out = pl.pallas_call(
        _kernel,
        grid=(1,),
        in_specs=[anyspec] * 8 + [pl.BlockSpec((1, M), lambda i: (0, 0))],
        out_specs=anyspec,
        out_shape=jax.ShapeDtypeStruct((S, M), BF16),
        scratch_shapes=[
            pltpu.VMEM((S // 2, M), U32), pltpu.VMEM((S // 2, DC), U32),
            pltpu.VMEM((H, M // 2, D), U32), pltpu.VMEM((H, DC // 2, D), U32), pltpu.VMEM((H, DC // 2, D), U32),
            pltpu.VMEM((H * D // 2, M), U32), pltpu.VMEM((M // 2, DB), U32), pltpu.VMEM((2, M // 2, DB), U32),
            pltpu.VMEM((DB // 2, DB), U32),
            pltpu.VMEM((S // 2, H * D), U32),
            pltpu.VMEM((S // 2, D), U32), pltpu.VMEM((S // 2, D), U32), pltpu.VMEM((S // 2, D), U32),
            pltpu.VMEM((2, S + PAD, DB), F32),
            pltpu.VMEM((NSLOT, M * H // NT1, D), BF16), pltpu.VMEM((NSLOT, DC * H // NT1, D), BF16),
            pltpu.VMEM((NSLOT, DC * H // NT1, D), BF16),
            pltpu.VMEM((NSLOT, RB, M), BF16), pltpu.VMEM((NSLOT, S // NT1, DC), BF16),
            pltpu.VMEM((2, M, DB), BF16),
            pltpu.VMEM((2, D, M), BF16), pltpu.VMEM((2, 32, DB), BF16), pltpu.VMEM((2, 32, DB), BF16),
            pltpu.VMEM((2, RB, M), BF16),
            pltpu.SemaphoreType.DMA((5, NSLOT)), pltpu.SemaphoreType.DMA((2,)),
            pltpu.SemaphoreType.DMA((3, 2)), pltpu.SemaphoreType.DMA((2,)),
        ],
        compiler_params=pltpu.CompilerParams(
            dimension_semantics=("arbitrary",), flags=FLAGS, vmem_limit_bytes=110 * 1024 * 1024),
    )(x, c, wq, wuk, wuv, wo, B_wqkv, B_wo, gw)
    return out.reshape(1, S, M)
```

```python
import functools
import jax
import jax.numpy as jnp
import jax.experimental.pallas as pl
import jax.experimental.pallas.tpu as pltpu

S = 2048
M = 1024
H = 32
D = 128
DC = 512
DB = 1024
W = 8
DIL = 2
BQ = 512
RB = 256
PAD = 16
NT1 = 16
NSLOT = 3
F32 = jnp.float32
BF16 = jnp.bfloat16
U32 = jnp.uint32
LOG2E = 1.4426950408889634
NEG = -1e30
NT = (((1,), (1,)), ((), ()))
FLAGS = {}
ORDER = lambda n: range(n - 1, -1, -1)
PCH = 8
P1SPLIT = 1
FINSPLIT = 2
KCH = 512


def _pk(v):
    return pltpu.bitcast(v.astype(BF16), U32)


def _up(u):
    return pltpu.bitcast(u, BF16)


def _rcp(l):
    r = pl.reciprocal(l, approx=True)
    return r * (2.0 - l * r)


def _swap_lane_tiles(u):
    lane = jax.lax.broadcasted_iota(jnp.int32, (u.shape[0], 128), 1)
    t = [u[:, i * 128:(i + 1) * 128] for i in range(8)]
    for b in range(3):
        s = 4 << b
        lo = (lane & s) == 0
        n = list(t)
        for i in range(8):
            if not (i >> b) & 1:
                A, B = t[i], t[i | (1 << b)]
                n[i] = jnp.where(lo, A, pltpu.roll(B, s, 1))
                n[i | (1 << b)] = jnp.where(lo, pltpu.roll(A, 128 - s, 1), B)
        t = n
    return jnp.concatenate(t, axis=1)


def _kernel(x_hbm, c_hbm, wq_hbm, wuk_hbm, wuv_hbm, wo_hbm, wqkv_hbm, wob_hbm, gate_ref,
            out_hbm,
            xu, cu, wq_u, wuk_u, wuv_u, wo_u, wqb_u, wkvb_u, wob_u, ctx_u, q_u, k_u, v_u,
            kvb_v, rq_v, ruk_v, ruv_v, rx_v, rc_v, rk_v, rv_v, jo_v, jq_v, jb_v, outs_v,
            rsem, wsem, vsem, jsem, osems):
    nrb = S // RB
    RQ = M * H // NT1
    RU = DC * H // NT1
    RC = S // NT1

    def x_cp(r, slot):
        return pltpu.make_async_copy(x_hbm.at[pl.ds(pl.multiple_of(r * RB, RB), RB), :], rx_v.at[slot], rsem.at[4, slot])

    def raw_cps(t, slot):
        return [
            pltpu.make_async_copy(wq_hbm.at[pl.ds(pl.multiple_of(t * RQ, RQ), RQ), :], rq_v.at[slot], rsem.at[0, slot]),
            pltpu.make_async_copy(wuk_hbm.at[pl.ds(pl.multiple_of(t * RU, RU), RU), :], ruk_v.at[slot], rsem.at[1, slot]),
            pltpu.make_async_copy(wuv_hbm.at[pl.ds(pl.multiple_of(t * RU, RU), RU), :], ruv_v.at[slot], rsem.at[2, slot]),
            pltpu.make_async_copy(c_hbm.at[pl.ds(pl.multiple_of(t * RC, RC), RC), :], rc_v.at[slot], rsem.at[3, slot]),
        ]

    def job_cps(h, slot):
        return [
            pltpu.make_async_copy(wo_hbm.at[pl.ds(pl.multiple_of(h * D, D), D), :], jo_v.at[slot], jsem.at[0, slot]),
            pltpu.make_async_copy(wqkv_hbm.at[pl.ds(pl.multiple_of(h * 32, 32), 32), pl.ds(0, DB)], jq_v.at[slot], jsem.at[1, slot]),
            pltpu.make_async_copy(wob_hbm.at[pl.ds(pl.multiple_of(h * 32, 32), 32), :], jb_v.at[slot], jsem.at[2, slot]),
        ]

    wk_cp = pltpu.make_async_copy(wqkv_hbm.at[:, pl.ds(DB, DB)], rk_v, wsem.at[0])
    VR = M // nrb

    def wv_cp(t):
        return pltpu.make_async_copy(wqkv_hbm.at[pl.ds(pl.multiple_of(t * VR, VR), VR), pl.ds(2 * DB, DB)],
                                     rv_v.at[t], vsem.at[t])

    def permute_k():
        lane = jax.lax.broadcasted_iota(jnp.int32, (PCH, 128), 1)
        for b in range(3):
            s = 4 << b
            lo = (lane & s) == 0
            for i in range(M // 2 // PCH):
                rs = slice(i * PCH, (i + 1) * PCH)
                for ta in range(8):
                    if (ta >> b) & 1:
                        continue
                    tb = ta | (1 << b)
                    ca, cb = slice(ta * 128, (ta + 1) * 128), slice(tb * 128, (tb + 1) * 128)
                    if b == 0:
                        A = _pk(rk_v[i * 2 * PCH:(i + 1) * 2 * PCH, ca])
                        B = _pk(rk_v[i * 2 * PCH:(i + 1) * 2 * PCH, cb])
                    else:
                        A, B = wkvb_u[0, rs, ca], wkvb_u[0, rs, cb]
                    wkvb_u[0, rs, ca] = jnp.where(lo, A, pltpu.roll(B, s, 1))
                    wkvb_u[0, rs, cb] = jnp.where(lo, pltpu.roll(A, 128 - s, 1), B)

    wk_cp.start()
    x_cp(0, 0).start()
    for c in raw_cps(0, 0):
        c.start()
    wv_cp(0).start()
    x_cp(1, 1).start()
    wv_cp(1).start()
    for c in raw_cps(1, 1):
        c.start()

    kvb_v[0, 0:PAD, :] = jnp.zeros((PAD, DB), F32)
    kvb_v[1, 0:PAD, :] = jnp.zeros((PAD, DB), F32)
    wk_cp.wait()
    permute_k()

    rq_u = rq_v.bitcast(U32)
    ruk_u = ruk_v.bitcast(U32)
    ruv_u = ruv_v.bitcast(U32)

    def relayout(src_u, slot, dst, row0, nrows, js):
        for j in js:
            u = src_u[slot, pl.ds(j, nrows, stride=H // 2), :]
            lo = pltpu.bitcast(u << 16, F32)
            hi = pltpu.bitcast(u & jnp.uint32(0xFFFF0000), F32)
            dst[2 * j, pl.ds(row0, nrows // 2), :] = _pk(lo)
            dst[2 * j + 1, pl.ds(row0, nrows // 2), :] = _pk(hi)

    def p1_body(t, carry):
        mat = t // nrb
        r = t % nrb
        slot = t % NSLOT

        @pl.when(t + 2 < NT1)
        def _():
            for c in raw_cps(t + 2, (t + 2) % NSLOT):
                c.start()

        @pl.when(t + 2 < nrb)
        def _():
            x_cp(t + 2, (t + 2) % NSLOT).start()

        @pl.when(t + 2 < nrb)
        def _():
            wv_cp(t + 2).start()

        @pl.when(t == NT1 - 2)
        def _():
            for c in job_cps(0, 0):
                c.start()

        @pl.when(t < nrb)
        def _():
            x_cp(t, slot).wait()
            xu[pl.ds(pl.multiple_of(t * (RB // 2), RB // 2), RB // 2), :] = _pk(rx_v[slot])

        @pl.when(t < nrb)
        def _():
            wv_cp(t).wait()

        for c in raw_cps(t, slot):
            c.wait()
        r0 = pl.multiple_of(r * RB, RB)
        hq = pl.multiple_of(t * (M // NT1 // 2), M // NT1 // 2)
        hu = pl.multiple_of(t * (DC // NT1 // 2), DC // NT1 // 2)
        xb = _up(xu[pl.ds(pl.multiple_of(r * (RB // 2), RB // 2), RB // 2), :])
        NP = P1SPLIT
        for p in range(NP):
            cs = slice(p * (DB // NP), (p + 1) * (DB // NP))
            kvb_v[mat, pl.ds(r0 + PAD, RB), cs] = jnp.dot(xb, _up(wkvb_u[mat, :, cs]), preferred_element_type=F32)
            js = range(p * (16 // NP), (p + 1) * (16 // NP))
            relayout(rq_u, slot, wq_u, hq, M // NT1, js)
            relayout(ruk_u, slot, wuk_u, hu, DC // NT1, js)
            relayout(ruv_u, slot, wuv_u, hu, DC // NT1, js)
        cu[pl.ds(pl.multiple_of(t * (RC // 2), RC // 2), RC // 2), :] = _pk(rc_v[slot])
        wkvb_u[1 + mat, pl.ds(pl.multiple_of(r * (VR // 2), VR // 2), VR // 2), :] = _swap_lane_tiles(_pk(rv_v[r]))
        return carry

    jax.lax.fori_loop(0, NT1, p1_body, 0)

    qscale = (D ** -0.5) * LOG2E

    def head_body(h, carry):
        js = h % 2

        @pl.when(h + 1 < H)
        def _():
            for c in job_cps(h + 1, 1 - js):
                c.start()

        for c in job_cps(h, js):
            c.wait()
        q = jnp.dot(_up(xu[...]), _up(wq_u[h]), preferred_element_type=F32)
        q_u[...] = _pk(q * qscale)
        cb = _up(cu[...])
        k_u[...] = _pk(jnp.dot(cb, _up(wuk_u[h]), preferred_element_type=F32))
        v_u[...] = _pk(jnp.dot(cb, _up(wuv_u[h]), preferred_element_type=F32))
        wo_u[pl.ds(pl.multiple_of(h * (D // 2), D // 2), D // 2), :] = _pk(jo_v[js])
        wqb_u[pl.ds(pl.multiple_of(h * 16, 16), 16), :] = _swap_lane_tiles(_pk(jq_v[js]))
        wob_u[pl.ds(pl.multiple_of(h * 16, 16), 16), :] = _pk(jb_v[js])
        lane0 = pl.multiple_of(h * D, D)
        tri = (jax.lax.broadcasted_iota(jnp.int32, (128, 128), 1)
               <= jax.lax.broadcasted_iota(jnp.int32, (128, 128), 0))
        for qi in ORDER(S // BQ):
            r0 = qi * BQ
            G = BQ // 128
            qb = _up(q_u[r0 // 2:(r0 + BQ) // 2, :])
            mt = None
            if qi > 0:
                sf = jax.lax.dot_general(qb, _up(k_u[0:r0 // 2, :]), NT, preferred_element_type=F32)
                mt = functools.reduce(jnp.maximum, [sf[:, t * 128:(t + 1) * 128] for t in range(r0 // 128)])
            sd = []
            for j in range(G):
                kj = _up(k_u[(r0 + j * 128) // 2:(r0 + (j + 1) * 128) // 2, :])
                sj = jax.lax.dot_general(qb[j * 128:], kj, NT, preferred_element_type=F32)
                top = jnp.where(tri, sj[:128], NEG)
                sd.append(top if j == G - 1 else jnp.concatenate([top, sj[128:]], axis=0))
            mg = []
            for i in range(G):
                ts = [sd[j][(i - j) * 128:(i - j + 1) * 128] for j in range(i + 1)]
                if mt is not None:
                    ts.append(mt[i * 128:(i + 1) * 128])
                mg.append(functools.reduce(jnp.maximum, ts))
            m = jnp.max(jnp.concatenate(mg, axis=0), axis=1, keepdims=True)
            pds = [jnp.exp2(sd[j] - m[j * 128:]) for j in range(G)]
            lg = []
            lt = None
            if qi > 0:
                pf = jnp.exp2(sf - m)
                lt = functools.reduce(jnp.add, [pf[:, t * 128:(t + 1) * 128] for t in range(r0 // 128)])
                acc = jnp.dot(pf.astype(BF16), _up(v_u[0:r0 // 2, :]), preferred_element_type=F32)
            for i in range(G):
                ts = [pds[j][(i - j) * 128:(i - j + 1) * 128] for j in range(i + 1)]
                if lt is not None:
                    ts.append(lt[i * 128:(i + 1) * 128])
                lg.append(functools.reduce(jnp.add, ts))
            l = jnp.sum(jnp.concatenate(lg, axis=0), axis=1, keepdims=True)
            accs = [jnp.dot(pds[j].astype(BF16), _up(v_u[(r0 + j * 128) // 2:(r0 + (j + 1) * 128) // 2, :]),
                            preferred_element_type=F32) for j in range(G)]
            rl = _rcp(l)
            for i in range(G):
                ts = [accs[j][(i - j) * 128:(i - j + 1) * 128] for j in range(i + 1)]
                if qi > 0:
                    ts.append(acc[i * 128:(i + 1) * 128])
                o = functools.reduce(jnp.add, ts) * rl[i * 128:(i + 1) * 128]
                ctx_u[(r0 + i * 128) // 2:(r0 + (i + 1) * 128) // 2, pl.ds(lane0, D)] = _pk(o)
        return carry

    jax.lax.fori_loop(0, H, head_body, 0)

    gw = gate_ref[...].astype(F32)
    bscale = (32 ** -0.5) * LOG2E

    def out_cp(r, slot):
        r0 = pl.multiple_of(r * RB, RB)
        return pltpu.make_async_copy(outs_v.at[slot], out_hbm.at[pl.ds(r0, RB), :], osems.at[slot])

    def fin_body(r, carry):
        r0 = pl.multiple_of(r * RB, RB)
        hr = pl.multiple_of(r * (RB // 2), RB // 2)
        slot = r % 2
        xb = _up(xu[pl.ds(hr, RB // 2), :])
        qb = jnp.dot(xb, _up(wqb_u[...]), preferred_element_type=F32) * bscale
        NS = FINSPLIT
        RS = RB // NS
        lane = jax.lax.broadcasted_iota(jnp.int32, (RS, 128), 1)
        odd1 = (lane & 1) == 1
        odd2 = (lane & 2) == 2
        a = None
        outs = []
        for sc in range(NS):
            s0 = sc * RS
            kw = kvb_v[0, pl.ds(r0 + s0, RS + PAD), :]
            vw = kvb_v[1, pl.ds(r0 + s0, RS + PAD), :]
            logits = []
            for w in range(W):
                o = PAD - DIL * w
                pr = qb[s0:s0 + RS] * kw[o:o + RS]
                lg = functools.reduce(jnp.add, [pr[:, t * 128:(t + 1) * 128] for t in range(8)])
                lg = lg + jnp.where(odd1, pltpu.roll(lg, 1, 1), pltpu.roll(lg, 127, 1))
                lg = lg + jnp.where(odd2, pltpu.roll(lg, 2, 1), pltpu.roll(lg, 126, 1))
                if w > 0 and s0 < PAD:
                    row = r0 + jax.lax.broadcasted_iota(jnp.int32, (PAD, 128), 0)
                    top = jnp.where(row >= DIL * w, lg[:PAD], NEG)
                    lg = top if RS == PAD else jnp.concatenate([top, lg[PAD:]], axis=0)
                logits.append(lg)
            for kc in range(sc * (8 // NS) * (512 // KCH), (sc + 1) * (8 // NS) * (512 // KCH)):
                ks = slice(kc * KCH, (kc + 1) * KCH)
                hs = slice(kc * KCH // 2, (kc + 1) * KCH // 2)
                at = jnp.dot(_up(ctx_u[pl.ds(hr, RB // 2), ks]), _up(wo_u[hs, :]), preferred_element_type=F32)
                a = at if a is None else a + at
            m = functools.reduce(jnp.maximum, logits)
            ps = [jnp.exp2(lg - m) for lg in logits]
            rl = _rcp(functools.reduce(jnp.add, ps))
            ps = [p * rl for p in ps]
            cols = []
            for t in range(8):
                cs = slice(t * 128, (t + 1) * 128)
                acc = None
                for w in range(W):
                    o = PAD - DIL * w
                    tt = ps[w] * vw[o:o + RS, cs]
                    acc = tt if acc is None else acc + tt
                cols.append(acc)
            outs.append(_swap_lane_tiles(_pk(jnp.concatenate(cols, axis=1))))
        ob = _up(jnp.concatenate(outs, axis=0))
        b = jnp.dot(ob, _up(wob_u[...]), preferred_element_type=F32)
        g = jax.nn.sigmoid(jnp.sum(xb.astype(F32) * gw, axis=1, keepdims=True))
        res = g * a + (1.0 - g) * b

        @pl.when(r >= 2)
        def _():
            out_cp(r - 2, slot).wait()

        outs_v[slot] = res.astype(BF16)
        out_cp(r, slot).start()
        return carry

    jax.lax.fori_loop(0, nrb, fin_body, 0)
    out_cp(nrb - 2, (nrb - 2) % 2).wait()
    out_cp(nrb - 1, (nrb - 1) % 2).wait()


@jax.jit
def pallas_gated_mix__compressed_kv_cla__sliding_local_dilated__prompt_kernel(
    A_x, A_c_kv, A_w_q, A_w_uk, A_w_uv, A_w_o, B_x, B_wqkv, B_wo, gate_w):
    x = A_x.reshape(S, M)
    c = A_c_kv.reshape(S, DC)
    wq = A_w_q.reshape(M * H, D)
    wuk = A_w_uk.reshape(DC * H, D)
    wuv = A_w_uv.reshape(DC * H, D)
    wo = A_w_o.reshape(H * D, M)
    gw = gate_w.reshape(1, M)
    anyspec = pl.BlockSpec(memory_space=pl.ANY)
    out = pl.pallas_call(
        _kernel,
        grid=(1,),
        in_specs=[anyspec] * 8 + [pl.BlockSpec((1, M), lambda i: (0, 0))],
        out_specs=anyspec,
        out_shape=jax.ShapeDtypeStruct((S, M), BF16),
        scratch_shapes=[
            pltpu.VMEM((S // 2, M), U32), pltpu.VMEM((S // 2, DC), U32),
            pltpu.VMEM((H, M // 2, D), U32), pltpu.VMEM((H, DC // 2, D), U32), pltpu.VMEM((H, DC // 2, D), U32),
            pltpu.VMEM((H * D // 2, M), U32), pltpu.VMEM((M // 2, DB), U32), pltpu.VMEM((3, M // 2, DB), U32),
            pltpu.VMEM((DB // 2, DB), U32),
            pltpu.VMEM((S // 2, H * D), U32),
            pltpu.VMEM((S // 2, D), U32), pltpu.VMEM((S // 2, D), U32), pltpu.VMEM((S // 2, D), U32),
            pltpu.VMEM((2, S + PAD, DB), F32),
            pltpu.VMEM((NSLOT, M * H // NT1, D), BF16), pltpu.VMEM((NSLOT, DC * H // NT1, D), BF16),
            pltpu.VMEM((NSLOT, DC * H // NT1, D), BF16),
            pltpu.VMEM((NSLOT, RB, M), BF16), pltpu.VMEM((NSLOT, S // NT1, DC), BF16),
            pltpu.VMEM((M, DB), BF16), pltpu.VMEM((S // RB, M // (S // RB), DB), BF16),
            pltpu.VMEM((2, D, M), BF16), pltpu.VMEM((2, 32, DB), BF16), pltpu.VMEM((2, 32, DB), BF16),
            pltpu.VMEM((2, RB, M), BF16),
            pltpu.SemaphoreType.DMA((5, NSLOT)), pltpu.SemaphoreType.DMA((1,)),
            pltpu.SemaphoreType.DMA((S // RB,)), pltpu.SemaphoreType.DMA((3, 2)), pltpu.SemaphoreType.DMA((2,)),
        ],
        compiler_params=pltpu.CompilerParams(
            dimension_semantics=("arbitrary",), flags=FLAGS, vmem_limit_bytes=110 * 1024 * 1024),
    )(x, c, wq, wuk, wuv, wo, B_wqkv, B_wo, gw)
    return out.reshape(1, S, M)
```

```python
import functools
import jax
import jax.numpy as jnp
import jax.experimental.pallas as pl
import jax.experimental.pallas.tpu as pltpu

S = 2048
M = 1024
H = 32
D = 128
DC = 512
DB = 1024
W = 8
DIL = 2
RB = 256
PAD = 16
NT1 = 16
NSLOT = 3
F32 = jnp.float32
BF16 = jnp.bfloat16
U32 = jnp.uint32
LOG2E = 1.4426950408889634
NEG = -1e30
NT = (((1,), (1,)), ((), ()))
FLAGS = {}
BLOCKS = [(1536, 512), (1024, 512), (512, 512), (0, 512)]
PCH = 8
P1SPLIT = 1
FINSPLIT = 2
KCH = 512


def _pk(v):
    return pltpu.bitcast(v.astype(BF16), U32)


def _up(u):
    return pltpu.bitcast(u, BF16)


def _rcp(l):
    r = pl.reciprocal(l, approx=True)
    return r * (2.0 - l * r)


def _swap_lane_tiles(u):
    lane = jax.lax.broadcasted_iota(jnp.int32, (u.shape[0], 128), 1)
    t = [u[:, i * 128:(i + 1) * 128] for i in range(8)]
    for b in range(3):
        s = 4 << b
        lo = (lane & s) == 0
        n = list(t)
        for i in range(8):
            if not (i >> b) & 1:
                A, B = t[i], t[i | (1 << b)]
                n[i] = jnp.where(lo, A, pltpu.roll(B, s, 1))
                n[i | (1 << b)] = jnp.where(lo, pltpu.roll(A, 128 - s, 1), B)
        t = n
    return jnp.concatenate(t, axis=1)


def _kernel(x_hbm, c_hbm, wq_hbm, wuk_hbm, wuv_hbm, wo_hbm, wqkv_hbm, wob_hbm, gate_ref,
            out_hbm,
            xu, cu, wq_u, wuk_u, wuv_u, wo_u, wqb_u, wkvb_u, wob_u, ctx_u, q_u, k_u, v_u,
            kvb_v, rq_v, ruk_v, ruv_v, rx_v, rc_v, rk_v, rv_v, jo_v, jq_v, jb_v, outs_v,
            rsem, wsem, vsem, jsem, osems):
    nrb = S // RB
    RQ = M * H // NT1
    RU = DC * H // NT1
    RC = S // NT1

    def x_cp(r, slot):
        return pltpu.make_async_copy(x_hbm.at[pl.ds(pl.multiple_of(r * RB, RB), RB), :], rx_v.at[slot], rsem.at[4, slot])

    def raw_cps(t, slot):
        return [
            pltpu.make_async_copy(wq_hbm.at[pl.ds(pl.multiple_of(t * RQ, RQ), RQ), :], rq_v.at[slot], rsem.at[0, slot]),
            pltpu.make_async_copy(wuk_hbm.at[pl.ds(pl.multiple_of(t * RU, RU), RU), :], ruk_v.at[slot], rsem.at[1, slot]),
            pltpu.make_async_copy(wuv_hbm.at[pl.ds(pl.multiple_of(t * RU, RU), RU), :], ruv_v.at[slot], rsem.at[2, slot]),
            pltpu.make_async_copy(c_hbm.at[pl.ds(pl.multiple_of(t * RC, RC), RC), :], rc_v.at[slot], rsem.at[3, slot]),
        ]

    def job_cps(h, slot):
        return [
            pltpu.make_async_copy(wo_hbm.at[pl.ds(pl.multiple_of(h * D, D), D), :], jo_v.at[slot], jsem.at[0, slot]),
            pltpu.make_async_copy(wqkv_hbm.at[pl.ds(pl.multiple_of(h * 32, 32), 32), pl.ds(0, DB)], jq_v.at[slot], jsem.at[1, slot]),
            pltpu.make_async_copy(wob_hbm.at[pl.ds(pl.multiple_of(h * 32, 32), 32), :], jb_v.at[slot], jsem.at[2, slot]),
        ]

    wk_cp = pltpu.make_async_copy(wqkv_hbm.at[:, pl.ds(DB, DB)], rk_v, wsem.at[0])
    VR = M // nrb

    def wv_cp(t):
        return pltpu.make_async_copy(wqkv_hbm.at[pl.ds(pl.multiple_of(t * VR, VR), VR), pl.ds(2 * DB, DB)],
                                     rv_v.at[t], vsem.at[t])

    def permute_k():
        lane = jax.lax.broadcasted_iota(jnp.int32, (PCH, 128), 1)
        for b in range(3):
            s = 4 << b
            lo = (lane & s) == 0
            for i in range(M // 2 // PCH):
                rs = slice(i * PCH, (i + 1) * PCH)
                for ta in range(8):
                    if (ta >> b) & 1:
                        continue
                    tb = ta | (1 << b)
                    ca, cb = slice(ta * 128, (ta + 1) * 128), slice(tb * 128, (tb + 1) * 128)
                    if b == 0:
                        A = _pk(rk_v[i * 2 * PCH:(i + 1) * 2 * PCH, ca])
                        B = _pk(rk_v[i * 2 * PCH:(i + 1) * 2 * PCH, cb])
                    else:
                        A, B = wkvb_u[0, rs, ca], wkvb_u[0, rs, cb]
                    wkvb_u[0, rs, ca] = jnp.where(lo, A, pltpu.roll(B, s, 1))
                    wkvb_u[0, rs, cb] = jnp.where(lo, pltpu.roll(A, 128 - s, 1), B)

    wk_cp.start()
    x_cp(0, 0).start()
    for c in raw_cps(0, 0):
        c.start()
    wv_cp(0).start()
    x_cp(1, 1).start()
    wv_cp(1).start()
    for c in raw_cps(1, 1):
        c.start()

    kvb_v[0, 0:PAD, :] = jnp.zeros((PAD, DB), F32)
    kvb_v[1, 0:PAD, :] = jnp.zeros((PAD, DB), F32)
    wk_cp.wait()
    permute_k()

    rq_u = rq_v.bitcast(U32)
    ruk_u = ruk_v.bitcast(U32)
    ruv_u = ruv_v.bitcast(U32)

    def relayout(src_u, slot, dst, row0, nrows, js):
        for j in js:
            u = src_u[slot, pl.ds(j, nrows, stride=H // 2), :]
            lo = pltpu.bitcast(u << 16, F32)
            hi = pltpu.bitcast(u & jnp.uint32(0xFFFF0000), F32)
            dst[2 * j, pl.ds(row0, nrows // 2), :] = _pk(lo)
            dst[2 * j + 1, pl.ds(row0, nrows // 2), :] = _pk(hi)

    def p1_body(t, carry):
        mat = t // nrb
        r = t % nrb
        slot = t % NSLOT

        @pl.when(t + 2 < NT1)
        def _():
            for c in raw_cps(t + 2, (t + 2) % NSLOT):
                c.start()

        @pl.when(t + 2 < nrb)
        def _():
            x_cp(t + 2, (t + 2) % NSLOT).start()

        @pl.when(t + 2 < nrb)
        def _():
            wv_cp(t + 2).start()

        @pl.when(t == NT1 - 2)
        def _():
            for c in job_cps(0, 0):
                c.start()

        @pl.when(t < nrb)
        def _():
            x_cp(t, slot).wait()
            xu[pl.ds(pl.multiple_of(t * (RB // 2), RB // 2), RB // 2), :] = _pk(rx_v[slot])

        @pl.when(t < nrb)
        def _():
            wv_cp(t).wait()

        for c in raw_cps(t, slot):
            c.wait()
        r0 = pl.multiple_of(r * RB, RB)
        hq = pl.multiple_of(t * (M // NT1 // 2), M // NT1 // 2)
        hu = pl.multiple_of(t * (DC // NT1 // 2), DC // NT1 // 2)
        xb = _up(xu[pl.ds(pl.multiple_of(r * (RB // 2), RB // 2), RB // 2), :])
        NP = P1SPLIT
        for p in range(NP):
            cs = slice(p * (DB // NP), (p + 1) * (DB // NP))
            kvb_v[mat, pl.ds(r0 + PAD, RB), cs] = jnp.dot(xb, _up(wkvb_u[mat, :, cs]), preferred_element_type=F32)
            js = range(p * (16 // NP), (p + 1) * (16 // NP))
            relayout(rq_u, slot, wq_u, hq, M // NT1, js)
            relayout(ruk_u, slot, wuk_u, hu, DC // NT1, js)
            relayout(ruv_u, slot, wuv_u, hu, DC // NT1, js)
        cu[pl.ds(pl.multiple_of(t * (RC // 2), RC // 2), RC // 2), :] = _pk(rc_v[slot])
        wkvb_u[1 + mat, pl.ds(pl.multiple_of(r * (VR // 2), VR // 2), VR // 2), :] = _swap_lane_tiles(_pk(rv_v[r]))
        return carry

    jax.lax.fori_loop(0, NT1, p1_body, 0)

    qscale = (D ** -0.5) * LOG2E

    def head_body(h, carry):
        js = h % 2

        @pl.when(h + 1 < H)
        def _():
            for c in job_cps(h + 1, 1 - js):
                c.start()

        for c in job_cps(h, js):
            c.wait()
        q = jnp.dot(_up(xu[...]), _up(wq_u[h]), preferred_element_type=F32)
        q_u[...] = _pk(q * qscale)
        cb = _up(cu[...])
        k_u[...] = _pk(jnp.dot(cb, _up(wuk_u[h]), preferred_element_type=F32))
        v_u[...] = _pk(jnp.dot(cb, _up(wuv_u[h]), preferred_element_type=F32))
        wo_u[pl.ds(pl.multiple_of(h * (D // 2), D // 2), D // 2), :] = _pk(jo_v[js])
        wqb_u[pl.ds(pl.multiple_of(h * 16, 16), 16), :] = _swap_lane_tiles(_pk(jq_v[js]))
        wob_u[pl.ds(pl.multiple_of(h * 16, 16), 16), :] = _pk(jb_v[js])
        lane0 = pl.multiple_of(h * D, D)
        tri = (jax.lax.broadcasted_iota(jnp.int32, (128, 128), 1)
               <= jax.lax.broadcasted_iota(jnp.int32, (128, 128), 0))
        for r0, BQ in BLOCKS:
            qi = r0
            G = BQ // 128
            qb = _up(q_u[r0 // 2:(r0 + BQ) // 2, :])
            mt = None
            if qi > 0:
                sf = jax.lax.dot_general(qb, _up(k_u[0:r0 // 2, :]), NT, preferred_element_type=F32)
                mt = functools.reduce(jnp.maximum, [sf[:, t * 128:(t + 1) * 128] for t in range(r0 // 128)])
            sd = []
            for j in range(G):
                kj = _up(k_u[(r0 + j * 128) // 2:(r0 + (j + 1) * 128) // 2, :])
                sj = jax.lax.dot_general(qb[j * 128:], kj, NT, preferred_element_type=F32)
                top = jnp.where(tri, sj[:128], NEG)
                sd.append(top if j == G - 1 else jnp.concatenate([top, sj[128:]], axis=0))
            mg = []
            for i in range(G):
                ts = [sd[j][(i - j) * 128:(i - j + 1) * 128] for j in range(i + 1)]
                if mt is not None:
                    ts.append(mt[i * 128:(i + 1) * 128])
                mg.append(functools.reduce(jnp.maximum, ts))
            m = jnp.max(jnp.concatenate(mg, axis=0), axis=1, keepdims=True)
            run = [None] * G
            lrun = [None] * G
            if qi > 0:
                pf = jnp.exp2(sf - m)
                lt = functools.reduce(jnp.add, [pf[:, t * 128:(t + 1) * 128] for t in range(r0 // 128)])
                acc = jnp.dot(pf.astype(BF16), _up(v_u[0:r0 // 2, :]), preferred_element_type=F32)
                run = [acc[i * 128:(i + 1) * 128] for i in range(G)]
                lrun = [lt[i * 128:(i + 1) * 128] for i in range(G)]
            for j in range(G):
                pj = jnp.exp2(sd[j] - m[j * 128:])
                aj = jnp.dot(pj.astype(BF16), _up(v_u[(r0 + j * 128) // 2:(r0 + (j + 1) * 128) // 2, :]),
                             preferred_element_type=F32)
                for i in range(j, G):
                    pa, pp = aj[(i - j) * 128:(i - j + 1) * 128], pj[(i - j) * 128:(i - j + 1) * 128]
                    run[i] = pa if run[i] is None else run[i] + pa
                    lrun[i] = pp if lrun[i] is None else lrun[i] + pp
                rl = _rcp(jnp.sum(lrun[j], axis=1, keepdims=True))
                ctx_u[(r0 + j * 128) // 2:(r0 + (j + 1) * 128) // 2, pl.ds(lane0, D)] = _pk(run[j] * rl)
        return carry

    jax.lax.fori_loop(0, H, head_body, 0)

    gw = gate_ref[...].astype(F32)
    bscale = (32 ** -0.5) * LOG2E

    def out_cp(r, slot):
        r0 = pl.multiple_of(r * RB, RB)
        return pltpu.make_async_copy(outs_v.at[slot], out_hbm.at[pl.ds(r0, RB), :], osems.at[slot])

    def fin_body(r, carry):
        r0 = pl.multiple_of(r * RB, RB)
        hr = pl.multiple_of(r * (RB // 2), RB // 2)
        slot = r % 2
        xb = _up(xu[pl.ds(hr, RB // 2), :])
        qb = jnp.dot(xb, _up(wqb_u[...]), preferred_element_type=F32) * bscale
        NS = FINSPLIT
        RS = RB // NS
        lane = jax.lax.broadcasted_iota(jnp.int32, (RS, 128), 1)
        odd1 = (lane & 1) == 1
        odd2 = (lane & 2) == 2
        a = None
        outs = []
        for sc in range(NS):
            s0 = sc * RS
            kw = kvb_v[0, pl.ds(r0 + s0, RS + PAD), :]
            vw = kvb_v[1, pl.ds(r0 + s0, RS + PAD), :]
            logits = []
            for w in range(W):
                o = PAD - DIL * w
                pr = qb[s0:s0 + RS] * kw[o:o + RS]
                lg = functools.reduce(jnp.add, [pr[:, t * 128:(t + 1) * 128] for t in range(8)])
                lg = lg + jnp.where(odd1, pltpu.roll(lg, 1, 1), pltpu.roll(lg, 127, 1))
                lg = lg + jnp.where(odd2, pltpu.roll(lg, 2, 1), pltpu.roll(lg, 126, 1))
                if w > 0 and s0 < PAD:
                    row = r0 + jax.lax.broadcasted_iota(jnp.int32, (PAD, 128), 0)
                    top = jnp.where(row >= DIL * w, lg[:PAD], NEG)
                    lg = top if RS == PAD else jnp.concatenate([top, lg[PAD:]], axis=0)
                logits.append(lg)
            for kc in range(sc * (8 // NS) * (512 // KCH), (sc + 1) * (8 // NS) * (512 // KCH)):
                ks = slice(kc * KCH, (kc + 1) * KCH)
                hs = slice(kc * KCH // 2, (kc + 1) * KCH // 2)
                at = jnp.dot(_up(ctx_u[pl.ds(hr, RB // 2), ks]), _up(wo_u[hs, :]), preferred_element_type=F32)
                a = at if a is None else a + at
            m = functools.reduce(jnp.maximum, logits)
            ps = [jnp.exp2(lg - m) for lg in logits]
            rl = _rcp(functools.reduce(jnp.add, ps))
            ps = [p * rl for p in ps]
            cols = []
            for t in range(8):
                cs = slice(t * 128, (t + 1) * 128)
                acc = None
                for w in range(W):
                    o = PAD - DIL * w
                    tt = ps[w] * vw[o:o + RS, cs]
                    acc = tt if acc is None else acc + tt
                cols.append(acc)
            outs.append(_swap_lane_tiles(_pk(jnp.concatenate(cols, axis=1))))
        ob = _up(jnp.concatenate(outs, axis=0))
        b = jnp.dot(ob, _up(wob_u[...]), preferred_element_type=F32)
        g = jax.nn.sigmoid(jnp.sum(xb.astype(F32) * gw, axis=1, keepdims=True))
        res = g * a + (1.0 - g) * b

        @pl.when(r >= 2)
        def _():
            out_cp(r - 2, slot).wait()

        outs_v[slot] = res.astype(BF16)
        out_cp(r, slot).start()
        return carry

    jax.lax.fori_loop(0, nrb, fin_body, 0)
    out_cp(nrb - 2, (nrb - 2) % 2).wait()
    out_cp(nrb - 1, (nrb - 1) % 2).wait()


@jax.jit
def pallas_gated_mix__compressed_kv_cla__sliding_local_dilated__prompt_kernel(
    A_x, A_c_kv, A_w_q, A_w_uk, A_w_uv, A_w_o, B_x, B_wqkv, B_wo, gate_w):
    x = A_x.reshape(S, M)
    c = A_c_kv.reshape(S, DC)
    wq = A_w_q.reshape(M * H, D)
    wuk = A_w_uk.reshape(DC * H, D)
    wuv = A_w_uv.reshape(DC * H, D)
    wo = A_w_o.reshape(H * D, M)
    gw = gate_w.reshape(1, M)
    anyspec = pl.BlockSpec(memory_space=pl.ANY)
    out = pl.pallas_call(
        _kernel,
        grid=(1,),
        in_specs=[anyspec] * 8 + [pl.BlockSpec((1, M), lambda i: (0, 0))],
        out_specs=anyspec,
        out_shape=jax.ShapeDtypeStruct((S, M), BF16),
        scratch_shapes=[
            pltpu.VMEM((S // 2, M), U32), pltpu.VMEM((S // 2, DC), U32),
            pltpu.VMEM((H, M // 2, D), U32), pltpu.VMEM((H, DC // 2, D), U32), pltpu.VMEM((H, DC // 2, D), U32),
            pltpu.VMEM((H * D // 2, M), U32), pltpu.VMEM((M // 2, DB), U32), pltpu.VMEM((3, M // 2, DB), U32),
            pltpu.VMEM((DB // 2, DB), U32),
            pltpu.VMEM((S // 2, H * D), U32),
            pltpu.VMEM((S // 2, D), U32), pltpu.VMEM((S // 2, D), U32), pltpu.VMEM((S // 2, D), U32),
            pltpu.VMEM((2, S + PAD, DB), F32),
            pltpu.VMEM((NSLOT, M * H // NT1, D), BF16), pltpu.VMEM((NSLOT, DC * H // NT1, D), BF16),
            pltpu.VMEM((NSLOT, DC * H // NT1, D), BF16),
            pltpu.VMEM((NSLOT, RB, M), BF16), pltpu.VMEM((NSLOT, S // NT1, DC), BF16),
            pltpu.VMEM((M, DB), BF16), pltpu.VMEM((S // RB, M // (S // RB), DB), BF16),
            pltpu.VMEM((2, D, M), BF16), pltpu.VMEM((2, 32, DB), BF16), pltpu.VMEM((2, 32, DB), BF16),
            pltpu.VMEM((2, RB, M), BF16),
            pltpu.SemaphoreType.DMA((5, NSLOT)), pltpu.SemaphoreType.DMA((1,)),
            pltpu.SemaphoreType.DMA((S // RB,)), pltpu.SemaphoreType.DMA((3, 2)), pltpu.SemaphoreType.DMA((2,)),
        ],
        compiler_params=pltpu.CompilerParams(
            dimension_semantics=("arbitrary",), flags=FLAGS, vmem_limit_bytes=110 * 1024 * 1024),
    )(x, c, wq, wuk, wuv, wo, B_wqkv, B_wo, gw)
    return out.reshape(1, S, M)
```

```python
import functools
import jax
import jax.numpy as jnp
import jax.experimental.pallas as pl
import jax.experimental.pallas.tpu as pltpu

S = 2048
M = 1024
H = 32
D = 128
DC = 512
DB = 1024
W = 8
DIL = 2
RF = 256
RB = 256
PAD = 16
NT1 = 16
NSLOT = 3
F32 = jnp.float32
BF16 = jnp.bfloat16
U32 = jnp.uint32
LOG2E = 1.4426950408889634
NEG = -1e30
NT = (((1,), (1,)), ((), ()))
FLAGS = {}
BLOCKS = [(1536, 512), (1024, 512), (512, 512), (0, 512)]
NKC = 8
P1ORD = 0
P1SPLIT = 1
FINSPLIT = 2
KCH = 512


def _pk(v):
    return pltpu.bitcast(v.astype(BF16), U32)


def _up(u):
    return pltpu.bitcast(u, BF16)


def _rcp(l):
    r = pl.reciprocal(l, approx=True)
    return r * (2.0 - l * r)


def _swap_lane_tiles(u):
    lane = jax.lax.broadcasted_iota(jnp.int32, (u.shape[0], 128), 1)
    t = [u[:, i * 128:(i + 1) * 128] for i in range(8)]
    for b in range(3):
        s = 4 << b
        lo = (lane & s) == 0
        n = list(t)
        for i in range(8):
            if not (i >> b) & 1:
                A, B = t[i], t[i | (1 << b)]
                n[i] = jnp.where(lo, A, pltpu.roll(B, s, 1))
                n[i | (1 << b)] = jnp.where(lo, pltpu.roll(A, 128 - s, 1), B)
        t = n
    return jnp.concatenate(t, axis=1)


def _kernel(x_hbm, c_hbm, wq_hbm, wuk_hbm, wuv_hbm, wo_hbm, wqkv_hbm, wob_hbm, gate_ref,
            out_hbm,
            xu, cu, wq_u, wuk_u, wuv_u, wo_u, wqb_u, wkvb_u, wob_u, ctx_u, q_u, k_u, v_u,
            kvb_v, rq_v, ruk_v, ruv_v, rx_v, rc_v, rk_v, rv_v, jo_v, jq_v, jb_v, outs_v,
            rsem, wsem, vsem, jsem, osems):
    nrb = S // RB
    RQ = M * H // NT1
    RU = DC * H // NT1
    RC = S // NT1

    def x_cp(r, slot):
        return pltpu.make_async_copy(x_hbm.at[pl.ds(pl.multiple_of(r * RB, RB), RB), :], rx_v.at[slot], rsem.at[4, slot])

    def raw_cps(t, slot):
        return [
            pltpu.make_async_copy(wq_hbm.at[pl.ds(pl.multiple_of(t * RQ, RQ), RQ), :], rq_v.at[slot], rsem.at[0, slot]),
            pltpu.make_async_copy(wuk_hbm.at[pl.ds(pl.multiple_of(t * RU, RU), RU), :], ruk_v.at[slot], rsem.at[1, slot]),
            pltpu.make_async_copy(wuv_hbm.at[pl.ds(pl.multiple_of(t * RU, RU), RU), :], ruv_v.at[slot], rsem.at[2, slot]),
            pltpu.make_async_copy(c_hbm.at[pl.ds(pl.multiple_of(t * RC, RC), RC), :], rc_v.at[slot], rsem.at[3, slot]),
        ]

    def job_cps(h, slot):
        return [
            pltpu.make_async_copy(wo_hbm.at[pl.ds(pl.multiple_of(h * D, D), D), :], jo_v.at[slot], jsem.at[0, slot]),
            pltpu.make_async_copy(wqkv_hbm.at[pl.ds(pl.multiple_of(h * 32, 32), 32), pl.ds(0, DB)], jq_v.at[slot], jsem.at[1, slot]),
            pltpu.make_async_copy(wob_hbm.at[pl.ds(pl.multiple_of(h * 32, 32), 32), :], jb_v.at[slot], jsem.at[2, slot]),
        ]

    KR = M // NKC

    def wk_cp(i):
        return pltpu.make_async_copy(wqkv_hbm.at[pl.ds(i * KR, KR), pl.ds(DB, DB)], rk_v.at[pl.ds(i * KR, KR), :], wsem.at[i])

    VR = M // nrb

    def wv_cp(t):
        return pltpu.make_async_copy(wqkv_hbm.at[pl.ds(pl.multiple_of(t * VR, VR), VR), pl.ds(2 * DB, DB)],
                                     rv_v.at[t], vsem.at[t])

    for i in range(NKC):
        wk_cp(i).start()
    x_cp(0, 0).start()
    for c in raw_cps(0, 0):
        c.start()
    wv_cp(0).start()
    x_cp(1, 1).start()
    wv_cp(1).start()
    for c in raw_cps(1, 1):
        c.start()

    kvb_v[0, 0:PAD, :] = jnp.zeros((PAD, DB), F32)
    kvb_v[1, 0:PAD, :] = jnp.zeros((PAD, DB), F32)
    for i in range(NKC):
        wk_cp(i).wait()
        wkvb_u[0, i * KR // 2:(i + 1) * KR // 2, :] = _swap_lane_tiles(_pk(rk_v[i * KR:(i + 1) * KR, :]))

    rq_u = rq_v.bitcast(U32)
    ruk_u = ruk_v.bitcast(U32)
    ruv_u = ruv_v.bitcast(U32)

    def relayout(src_u, slot, dst, row0, nrows, js):
        for j in js:
            u = src_u[slot, pl.ds(j, nrows, stride=H // 2), :]
            lo = pltpu.bitcast(u << 16, F32)
            hi = pltpu.bitcast(u & jnp.uint32(0xFFFF0000), F32)
            dst[2 * j, pl.ds(row0, nrows // 2), :] = _pk(lo)
            dst[2 * j + 1, pl.ds(row0, nrows // 2), :] = _pk(hi)

    def p1_body(t, carry):
        mat = t // nrb
        r = t % nrb
        slot = t % NSLOT

        @pl.when(t + 2 < NT1)
        def _():
            for c in raw_cps(t + 2, (t + 2) % NSLOT):
                c.start()

        @pl.when(t + 2 < nrb)
        def _():
            x_cp(t + 2, (t + 2) % NSLOT).start()

        @pl.when(t + 2 < nrb)
        def _():
            wv_cp(t + 2).start()

        @pl.when(t == NT1 - 2)
        def _():
            for c in job_cps(0, 0):
                c.start()

        @pl.when(t < nrb)
        def _():
            x_cp(t, slot).wait()
            xu[pl.ds(pl.multiple_of(t * (RB // 2), RB // 2), RB // 2), :] = _pk(rx_v[slot])

        @pl.when(t < nrb)
        def _():
            wv_cp(t).wait()

        for c in raw_cps(t, slot):
            c.wait()
        r0 = pl.multiple_of(r * RB, RB)
        hq = pl.multiple_of(t * (M // NT1 // 2), M // NT1 // 2)
        hu = pl.multiple_of(t * (DC // NT1 // 2), DC // NT1 // 2)
        xb = _up(xu[pl.ds(pl.multiple_of(r * (RB // 2), RB // 2), RB // 2), :])
        def st_mm():
            kvb_v[mat, pl.ds(r0 + PAD, RB), :] = jnp.dot(xb, _up(wkvb_u[mat]), preferred_element_type=F32)

        def st_rq():
            relayout(rq_u, slot, wq_u, hq, M // NT1, range(16))

        def st_ru():
            relayout(ruk_u, slot, wuk_u, hu, DC // NT1, range(16))
            relayout(ruv_u, slot, wuv_u, hu, DC // NT1, range(16))

        def st_c():
            cu[pl.ds(pl.multiple_of(t * (RC // 2), RC // 2), RC // 2), :] = _pk(rc_v[slot])

        def st_wv():
            wkvb_u[1 + mat, pl.ds(pl.multiple_of(r * (VR // 2), VR // 2), VR // 2), :] = _swap_lane_tiles(_pk(rv_v[r]))

        stages = [[st_mm, st_rq, st_ru, st_c, st_wv], [st_wv, st_c, st_mm, st_rq, st_ru], [st_rq, st_ru, st_c, st_wv, st_mm],
                  [st_wv, st_mm, st_ru, st_rq, st_c], [st_c, st_rq, st_mm, st_ru, st_wv]][P1ORD]
        for st in stages:
            st()
        return carry

    jax.lax.fori_loop(0, NT1, p1_body, 0)

    qscale = (D ** -0.5) * LOG2E

    def head_body(h, carry):
        js = h % 2

        @pl.when(h + 1 < H)
        def _():
            for c in job_cps(h + 1, 1 - js):
                c.start()

        for c in job_cps(h, js):
            c.wait()
        q = jnp.dot(_up(xu[...]), _up(wq_u[h]), preferred_element_type=F32)
        q_u[...] = _pk(q * qscale)
        cb = _up(cu[...])
        k_u[...] = _pk(jnp.dot(cb, _up(wuk_u[h]), preferred_element_type=F32))
        v_u[...] = _pk(jnp.dot(cb, _up(wuv_u[h]), preferred_element_type=F32))
        wo_u[pl.ds(pl.multiple_of(h * (D // 2), D // 2), D // 2), :] = _pk(jo_v[js])
        wqb_u[pl.ds(pl.multiple_of(h * 16, 16), 16), :] = _swap_lane_tiles(_pk(jq_v[js]))
        wob_u[pl.ds(pl.multiple_of(h * 16, 16), 16), :] = _pk(jb_v[js])
        lane0 = pl.multiple_of(h * D, D)
        tri = (jax.lax.broadcasted_iota(jnp.int32, (128, 128), 1)
               <= jax.lax.broadcasted_iota(jnp.int32, (128, 128), 0))
        for r0, BQ in BLOCKS:
            qi = r0
            G = BQ // 128
            qb = _up(q_u[r0 // 2:(r0 + BQ) // 2, :])
            mt = None
            if qi > 0:
                sf = jax.lax.dot_general(qb, _up(k_u[0:r0 // 2, :]), NT, preferred_element_type=F32)
                mt = functools.reduce(jnp.maximum, [sf[:, t * 128:(t + 1) * 128] for t in range(r0 // 128)])
            sd = []
            for j in range(G):
                kj = _up(k_u[(r0 + j * 128) // 2:(r0 + (j + 1) * 128) // 2, :])
                sj = jax.lax.dot_general(qb[j * 128:], kj, NT, preferred_element_type=F32)
                top = jnp.where(tri, sj[:128], NEG)
                sd.append(top if j == G - 1 else jnp.concatenate([top, sj[128:]], axis=0))
            mg = []
            for i in range(G):
                ts = [sd[j][(i - j) * 128:(i - j + 1) * 128] for j in range(i + 1)]
                if mt is not None:
                    ts.append(mt[i * 128:(i + 1) * 128])
                mg.append(functools.reduce(jnp.maximum, ts))
            m = jnp.max(jnp.concatenate(mg, axis=0), axis=1, keepdims=True)
            run = [None] * G
            lrun = [None] * G
            if qi > 0:
                pf = jnp.exp2(sf - m)
                lt = functools.reduce(jnp.add, [pf[:, t * 128:(t + 1) * 128] for t in range(r0 // 128)])
                acc = jnp.dot(pf.astype(BF16), _up(v_u[0:r0 // 2, :]), preferred_element_type=F32)
                run = [acc[i * 128:(i + 1) * 128] for i in range(G)]
                lrun = [lt[i * 128:(i + 1) * 128] for i in range(G)]
            for j in range(G):
                pj = jnp.exp2(sd[j] - m[j * 128:])
                aj = jnp.dot(pj.astype(BF16), _up(v_u[(r0 + j * 128) // 2:(r0 + (j + 1) * 128) // 2, :]),
                             preferred_element_type=F32)
                for i in range(j, G):
                    pa, pp = aj[(i - j) * 128:(i - j + 1) * 128], pj[(i - j) * 128:(i - j + 1) * 128]
                    run[i] = pa if run[i] is None else run[i] + pa
                    lrun[i] = pp if lrun[i] is None else lrun[i] + pp
                rl = _rcp(jnp.sum(lrun[j], axis=1, keepdims=True))
                ctx_u[(r0 + j * 128) // 2:(r0 + (j + 1) * 128) // 2, pl.ds(lane0, D)] = _pk(run[j] * rl)
        return carry

    jax.lax.fori_loop(0, H, head_body, 0)

    gw = gate_ref[...].astype(F32)
    bscale = (32 ** -0.5) * LOG2E

    nrf = S // RF

    def out_cp(r, slot):
        r0 = pl.multiple_of(r * RF, RF)
        return pltpu.make_async_copy(outs_v.at[slot], out_hbm.at[pl.ds(r0, RF), :], osems.at[slot])

    def fin_body(r, carry):
        r0 = pl.multiple_of(r * RF, RF)
        hr = pl.multiple_of(r * (RF // 2), RF // 2)
        slot = r % 2
        xb = _up(xu[pl.ds(hr, RF // 2), :])
        qb = jnp.dot(xb, _up(wqb_u[...]), preferred_element_type=F32) * bscale
        NS = FINSPLIT
        RS = RF // NS
        lane = jax.lax.broadcasted_iota(jnp.int32, (RS, 128), 1)
        odd1 = (lane & 1) == 1
        odd2 = (lane & 2) == 2
        a = None
        outs = []
        for sc in range(NS):
            s0 = sc * RS
            kw = kvb_v[0, pl.ds(r0 + s0, RS + PAD), :]
            vw = kvb_v[1, pl.ds(r0 + s0, RS + PAD), :]
            logits = []
            for w in range(W):
                o = PAD - DIL * w
                pr = qb[s0:s0 + RS] * kw[o:o + RS]
                lg = functools.reduce(jnp.add, [pr[:, t * 128:(t + 1) * 128] for t in range(8)])
                lg = lg + jnp.where(odd1, pltpu.roll(lg, 1, 1), pltpu.roll(lg, 127, 1))
                lg = lg + jnp.where(odd2, pltpu.roll(lg, 2, 1), pltpu.roll(lg, 126, 1))
                if w > 0 and s0 < PAD:
                    row = r0 + jax.lax.broadcasted_iota(jnp.int32, (PAD, 128), 0)
                    top = jnp.where(row >= DIL * w, lg[:PAD], NEG)
                    lg = top if RS == PAD else jnp.concatenate([top, lg[PAD:]], axis=0)
                logits.append(lg)
            for kc in range(sc * (H * D // KCH) // NS, (sc + 1) * (H * D // KCH) // NS):
                ks = slice(kc * KCH, (kc + 1) * KCH)
                hs = slice(kc * KCH // 2, (kc + 1) * KCH // 2)
                at = jnp.dot(_up(ctx_u[pl.ds(hr, RF // 2), ks]), _up(wo_u[hs, :]), preferred_element_type=F32)
                a = at if a is None else a + at
            m = functools.reduce(jnp.maximum, logits)
            ps = [jnp.exp2(lg - m) for lg in logits]
            rl = _rcp(functools.reduce(jnp.add, ps))
            ps = [p * rl for p in ps]
            cols = []
            for t in range(8):
                cs = slice(t * 128, (t + 1) * 128)
                acc = None
                for w in range(W):
                    o = PAD - DIL * w
                    tt = ps[w] * vw[o:o + RS, cs]
                    acc = tt if acc is None else acc + tt
                cols.append(acc)
            outs.append(_swap_lane_tiles(_pk(jnp.concatenate(cols, axis=1))))
        ob = _up(jnp.concatenate(outs, axis=0))
        b = jnp.dot(ob, _up(wob_u[...]), preferred_element_type=F32)
        g = jax.nn.sigmoid(jnp.sum(xb.astype(F32) * gw, axis=1, keepdims=True))
        res = g * a + (1.0 - g) * b

        @pl.when(r >= 2)
        def _():
            out_cp(r - 2, slot).wait()

        outs_v[slot] = res.astype(BF16)
        out_cp(r, slot).start()
        return carry

    jax.lax.fori_loop(0, nrf, fin_body, 0)
    out_cp(nrf - 2, (nrf - 2) % 2).wait()
    out_cp(nrf - 1, (nrf - 1) % 2).wait()


@jax.jit
def pallas_gated_mix__compressed_kv_cla__sliding_local_dilated__prompt_kernel(
    A_x, A_c_kv, A_w_q, A_w_uk, A_w_uv, A_w_o, B_x, B_wqkv, B_wo, gate_w):
    x = A_x.reshape(S, M)
    c = A_c_kv.reshape(S, DC)
    wq = A_w_q.reshape(M * H, D)
    wuk = A_w_uk.reshape(DC * H, D)
    wuv = A_w_uv.reshape(DC * H, D)
    wo = A_w_o.reshape(H * D, M)
    gw = gate_w.reshape(1, M)
    anyspec = pl.BlockSpec(memory_space=pl.ANY)
    out = pl.pallas_call(
        _kernel,
        grid=(1,),
        in_specs=[anyspec] * 8 + [pl.BlockSpec((1, M), lambda i: (0, 0))],
        out_specs=anyspec,
        out_shape=jax.ShapeDtypeStruct((S, M), BF16),
        scratch_shapes=[
            pltpu.VMEM((S // 2, M), U32), pltpu.VMEM((S // 2, DC), U32),
            pltpu.VMEM((H, M // 2, D), U32), pltpu.VMEM((H, DC // 2, D), U32), pltpu.VMEM((H, DC // 2, D), U32),
            pltpu.VMEM((H * D // 2, M), U32), pltpu.VMEM((M // 2, DB), U32), pltpu.VMEM((3, M // 2, DB), U32),
            pltpu.VMEM((DB // 2, DB), U32),
            pltpu.VMEM((S // 2, H * D), U32),
            pltpu.VMEM((S // 2, D), U32), pltpu.VMEM((S // 2, D), U32), pltpu.VMEM((S // 2, D), U32),
            pltpu.VMEM((2, S + PAD, DB), F32),
            pltpu.VMEM((NSLOT, M * H // NT1, D), BF16), pltpu.VMEM((NSLOT, DC * H // NT1, D), BF16),
            pltpu.VMEM((NSLOT, DC * H // NT1, D), BF16),
            pltpu.VMEM((NSLOT, RB, M), BF16), pltpu.VMEM((NSLOT, S // NT1, DC), BF16),
            pltpu.VMEM((M, DB), BF16), pltpu.VMEM((S // RB, M // (S // RB), DB), BF16),
            pltpu.VMEM((2, D, M), BF16), pltpu.VMEM((2, 32, DB), BF16), pltpu.VMEM((2, 32, DB), BF16),
            pltpu.VMEM((2, RF, M), BF16),
            pltpu.SemaphoreType.DMA((5, NSLOT)), pltpu.SemaphoreType.DMA((NKC,)),
            pltpu.SemaphoreType.DMA((S // RB,)), pltpu.SemaphoreType.DMA((3, 2)), pltpu.SemaphoreType.DMA((2,)),
        ],
        compiler_params=pltpu.CompilerParams(
            dimension_semantics=("arbitrary",), flags=FLAGS, vmem_limit_bytes=110 * 1024 * 1024),
    )(x, c, wq, wuk, wuv, wo, B_wqkv, B_wo, gw)
    return out.reshape(1, S, M)
```

```python
import functools
import jax
import jax.numpy as jnp
import jax.experimental.pallas as pl
import jax.experimental.pallas.tpu as pltpu

S = 2048
M = 1024
H = 32
D = 128
DC = 512
DB = 1024
W = 8
DIL = 2
RF = 256
RB = 256
PAD = 16
NT1 = 16
NSLOT = 3
F32 = jnp.float32
BF16 = jnp.bfloat16
U32 = jnp.uint32
LOG2E = 1.4426950408889634
NEG = -1e9 * LOG2E
NT = (((1,), (1,)), ((), ()))
BLOCKS = [(1536, 512), (1024, 512), (512, 512), (0, 512)]
NKC = 8
FINSPLIT = 2
KCH = 512


def _pk(v):
    return pltpu.bitcast(v.astype(BF16), U32)


def _up(u):
    return pltpu.bitcast(u, BF16)


def _rcp(l):
    r = pl.reciprocal(l, approx=True)
    return r * (2.0 - l * r)


def _swap_lane_tiles(u):
    lane = jax.lax.broadcasted_iota(jnp.int32, (u.shape[0], 128), 1)
    t = [u[:, i * 128:(i + 1) * 128] for i in range(8)]
    for b in range(3):
        s = 4 << b
        lo = (lane & s) == 0
        n = list(t)
        for i in range(8):
            if not (i >> b) & 1:
                A, B = t[i], t[i | (1 << b)]
                n[i] = jnp.where(lo, A, pltpu.roll(B, s, 1))
                n[i | (1 << b)] = jnp.where(lo, pltpu.roll(A, 128 - s, 1), B)
        t = n
    return jnp.concatenate(t, axis=1)


def _kernel(x_hbm, c_hbm, wq_hbm, wuk_hbm, wuv_hbm, wo_hbm, wqkv_hbm, wob_hbm, gate_ref,
            out_hbm,
            xu, cu, wq_u, wuk_u, wuv_u, wo_u, wqb_u, wk_u, wv_u, wob_u, ctx_u, q_u, k_u, v_u,
            kvb_v, rq_v, ruk_v, ruv_v, rx_v, rc_v, rk_v, rv_v, jo_v, jq_v, jb_v, outs_v,
            rsem, wsem, vsem, jsem, osems):
    nrb = S // RB
    RQ = M * H // NT1
    RU = DC * H // NT1
    RC = S // NT1

    def x_cp(r, slot):
        return pltpu.make_async_copy(x_hbm.at[pl.ds(pl.multiple_of(r * RB, RB), RB), :], rx_v.at[slot], rsem.at[4, slot])

    def raw_cps(t, slot):
        return [
            pltpu.make_async_copy(wq_hbm.at[pl.ds(pl.multiple_of(t * RQ, RQ), RQ), :], rq_v.at[slot], rsem.at[0, slot]),
            pltpu.make_async_copy(wuk_hbm.at[pl.ds(pl.multiple_of(t * RU, RU), RU), :], ruk_v.at[slot], rsem.at[1, slot]),
            pltpu.make_async_copy(wuv_hbm.at[pl.ds(pl.multiple_of(t * RU, RU), RU), :], ruv_v.at[slot], rsem.at[2, slot]),
            pltpu.make_async_copy(c_hbm.at[pl.ds(pl.multiple_of(t * RC, RC), RC), :], rc_v.at[slot], rsem.at[3, slot]),
        ]

    def job_cps(h, slot):
        return [
            pltpu.make_async_copy(wo_hbm.at[pl.ds(pl.multiple_of(h * D, D), D), :], jo_v.at[slot], jsem.at[0, slot]),
            pltpu.make_async_copy(wqkv_hbm.at[pl.ds(pl.multiple_of(h * 32, 32), 32), pl.ds(0, DB)], jq_v.at[slot], jsem.at[1, slot]),
            pltpu.make_async_copy(wob_hbm.at[pl.ds(pl.multiple_of(h * 32, 32), 32), :], jb_v.at[slot], jsem.at[2, slot]),
        ]

    KR = M // NKC

    def wk_cp(i):
        return pltpu.make_async_copy(wqkv_hbm.at[pl.ds(i * KR, KR), pl.ds(DB, DB)], rk_v.at[pl.ds(i * KR, KR), :], wsem.at[i])

    VR = M // nrb

    def wv_cp(t):
        return pltpu.make_async_copy(wqkv_hbm.at[pl.ds(pl.multiple_of(t * VR, VR), VR), pl.ds(2 * DB, DB)],
                                     rv_v.at[t], vsem.at[t])

    for i in range(NKC):
        wk_cp(i).start()
    x_cp(0, 0).start()
    for c in raw_cps(0, 0):
        c.start()
    wv_cp(0).start()
    x_cp(1, 1).start()
    wv_cp(1).start()
    for c in raw_cps(1, 1):
        c.start()

    kvb_v[0, 0:PAD, :] = jnp.zeros((PAD, DB), F32)
    kvb_v[1, 0:PAD, :] = jnp.zeros((PAD, DB), F32)
    for i in range(NKC):
        wk_cp(i).wait()
        wk_u[i * KR // 2:(i + 1) * KR // 2, :] = _swap_lane_tiles(_pk(rk_v[i * KR:(i + 1) * KR, :]))

    rq_u = rq_v.bitcast(U32)
    ruk_u = ruk_v.bitcast(U32)
    ruv_u = ruv_v.bitcast(U32)

    def relayout(src_u, slot, dst, row0, nrows):
        for j in range(H // 2):
            u = src_u[slot, pl.ds(j, nrows, stride=H // 2), :]
            lo = pltpu.bitcast(u << 16, F32)
            hi = pltpu.bitcast(u & jnp.uint32(0xFFFF0000), F32)
            dst[2 * j, pl.ds(row0, nrows // 2), :] = _pk(lo)
            dst[2 * j + 1, pl.ds(row0, nrows // 2), :] = _pk(hi)

    def p1_body(mat, r, carry):
        t = mat * nrb + r
        slot = t % NSLOT

        @pl.when(t + 2 < NT1)
        def _():
            for c in raw_cps(t + 2, (t + 2) % NSLOT):
                c.start()

        if mat == 0:
            @pl.when(r + 2 < nrb)
            def _():
                x_cp(r + 2, (r + 2) % NSLOT).start()
                wv_cp(r + 2).start()

            x_cp(r, slot).wait()
            wv_cp(r).wait()
        else:
            @pl.when(r == nrb - 2)
            def _():
                for c in job_cps(0, 0):
                    c.start()

        for c in raw_cps(t, slot):
            c.wait()
        r0 = pl.multiple_of(r * RB, RB)
        hx = pl.multiple_of(r * (RB // 2), RB // 2)
        hq = pl.multiple_of(t * (M // NT1 // 2), M // NT1 // 2)
        hu = pl.multiple_of(t * (DC // NT1 // 2), DC // NT1 // 2)
        xb = rx_v[slot] if mat == 0 else _up(xu[pl.ds(hx, RB // 2), :])
        w_u = wk_u if mat == 0 else wv_u

        kvb_v[mat, pl.ds(r0 + PAD, RB), :] = jnp.dot(xb, _up(w_u[...]), preferred_element_type=F32)
        relayout(rq_u, slot, wq_u, hq, M // NT1)
        relayout(ruk_u, slot, wuk_u, hu, DC // NT1)
        relayout(ruv_u, slot, wuv_u, hu, DC // NT1)
        cu[pl.ds(pl.multiple_of(t * (RC // 2), RC // 2), RC // 2), :] = _pk(rc_v[slot])
        if mat == 0:
            wv_u[pl.ds(pl.multiple_of(r * (VR // 2), VR // 2), VR // 2), :] = _swap_lane_tiles(_pk(rv_v[r]))
            xu[pl.ds(hx, RB // 2), :] = _pk(xb)
        return carry

    jax.lax.fori_loop(0, nrb, functools.partial(p1_body, 0), 0)
    jax.lax.fori_loop(0, nrb, functools.partial(p1_body, 1), 0)

    qscale = (D ** -0.5) * LOG2E

    def head_body(h, carry):
        js = h % 2

        @pl.when(h + 1 < H)
        def _():
            for c in job_cps(h + 1, 1 - js):
                c.start()

        for c in job_cps(h, js):
            c.wait()
        q = jnp.dot(_up(xu[...]), _up(wq_u[h]), preferred_element_type=F32)
        q_u[...] = _pk(q * qscale)
        cb = _up(cu[...])
        k_u[...] = _pk(jnp.dot(cb, _up(wuk_u[h]), preferred_element_type=F32))
        v_u[...] = _pk(jnp.dot(cb, _up(wuv_u[h]), preferred_element_type=F32))
        wo_u[pl.ds(pl.multiple_of(h * (D // 2), D // 2), D // 2), :] = _pk(jo_v[js])
        wqb_u[pl.ds(pl.multiple_of(h * 16, 16), 16), :] = _swap_lane_tiles(_pk(jq_v[js]))
        wob_u[pl.ds(pl.multiple_of(h * 16, 16), 16), :] = _pk(jb_v[js])
        lane0 = pl.multiple_of(h * D, D)
        tri = (jax.lax.broadcasted_iota(jnp.int32, (128, 128), 1)
               <= jax.lax.broadcasted_iota(jnp.int32, (128, 128), 0))
        for r0, BQ in BLOCKS:
            G = BQ // 128
            qb = _up(q_u[r0 // 2:(r0 + BQ) // 2, :])
            mt = None
            if r0 > 0:
                sf = jax.lax.dot_general(qb, _up(k_u[0:r0 // 2, :]), NT, preferred_element_type=F32)
                mt = functools.reduce(jnp.maximum, [sf[:, t * 128:(t + 1) * 128] for t in range(r0 // 128)])
            sd = []
            for j in range(G):
                kj = _up(k_u[(r0 + j * 128) // 2:(r0 + (j + 1) * 128) // 2, :])
                sj = jax.lax.dot_general(qb[j * 128:], kj, NT, preferred_element_type=F32)
                top = jnp.where(tri, sj[:128], NEG)
                sd.append(top if j == G - 1 else jnp.concatenate([top, sj[128:]], axis=0))
            mg = []
            for i in range(G):
                ts = [sd[j][(i - j) * 128:(i - j + 1) * 128] for j in range(i + 1)]
                if mt is not None:
                    ts.append(mt[i * 128:(i + 1) * 128])
                mg.append(functools.reduce(jnp.maximum, ts))
            m = jnp.max(jnp.concatenate(mg, axis=0), axis=1, keepdims=True)
            run = [None] * G
            lrun = [None] * G
            if r0 > 0:
                pf = jnp.exp2(sf - m)
                lt = functools.reduce(jnp.add, [pf[:, t * 128:(t + 1) * 128] for t in range(r0 // 128)])
                acc = jnp.dot(pf.astype(BF16), _up(v_u[0:r0 // 2, :]), preferred_element_type=F32)
                run = [acc[i * 128:(i + 1) * 128] for i in range(G)]
                lrun = [lt[i * 128:(i + 1) * 128] for i in range(G)]
            for j in range(G):
                pj = jnp.exp2(sd[j] - m[j * 128:])
                aj = jnp.dot(pj.astype(BF16), _up(v_u[(r0 + j * 128) // 2:(r0 + (j + 1) * 128) // 2, :]),
                             preferred_element_type=F32)
                for i in range(j, G):
                    pa, pp = aj[(i - j) * 128:(i - j + 1) * 128], pj[(i - j) * 128:(i - j + 1) * 128]
                    run[i] = pa if run[i] is None else run[i] + pa
                    lrun[i] = pp if lrun[i] is None else lrun[i] + pp
                rl = _rcp(jnp.sum(lrun[j], axis=1, keepdims=True))
                ctx_u[(r0 + j * 128) // 2:(r0 + (j + 1) * 128) // 2, pl.ds(lane0, D)] = _pk(run[j] * rl)
        return carry

    jax.lax.fori_loop(0, H, head_body, 0)

    gw = gate_ref[...].astype(F32)[None, :]
    bscale = (32 ** -0.5) * LOG2E

    nrf = S // RF

    def out_cp(r, slot):
        r0 = pl.multiple_of(r * RF, RF)
        return pltpu.make_async_copy(outs_v.at[slot], out_hbm.at[pl.ds(r0, RF), :], osems.at[slot])

    def fin_body(r, carry):
        r0 = pl.multiple_of(r * RF, RF)
        hr = pl.multiple_of(r * (RF // 2), RF // 2)
        slot = r % 2
        xb = _up(xu[pl.ds(hr, RF // 2), :])
        qb = jnp.dot(xb, _up(wqb_u[...]), preferred_element_type=F32) * bscale
        NS = FINSPLIT
        RS = RF // NS
        lane = jax.lax.broadcasted_iota(jnp.int32, (RS, 128), 1)
        odd1 = (lane & 1) == 1
        odd2 = (lane & 2) == 2
        a = None
        outs = []
        for sc in range(NS):
            s0 = sc * RS
            kw = kvb_v[0, pl.ds(r0 + s0, RS + PAD), :]
            vw = kvb_v[1, pl.ds(r0 + s0, RS + PAD), :]
            logits = []
            for w in range(W):
                o = PAD - DIL * w
                pr = qb[s0:s0 + RS] * kw[o:o + RS]
                lg = functools.reduce(jnp.add, [pr[:, t * 128:(t + 1) * 128] for t in range(8)])
                lg = lg + jnp.where(odd1, pltpu.roll(lg, 1, 1), pltpu.roll(lg, 127, 1))
                lg = lg + jnp.where(odd2, pltpu.roll(lg, 2, 1), pltpu.roll(lg, 126, 1))
                if w > 0 and s0 < PAD:
                    row = r0 + jax.lax.broadcasted_iota(jnp.int32, (PAD, 128), 0)
                    top = jnp.where(row >= DIL * w, lg[:PAD], NEG)
                    lg = top if RS == PAD else jnp.concatenate([top, lg[PAD:]], axis=0)
                logits.append(lg)
            for kc in range(sc * (H * D // KCH) // NS, (sc + 1) * (H * D // KCH) // NS):
                ks = slice(kc * KCH, (kc + 1) * KCH)
                hs = slice(kc * KCH // 2, (kc + 1) * KCH // 2)
                at = jnp.dot(_up(ctx_u[pl.ds(hr, RF // 2), ks]), _up(wo_u[hs, :]), preferred_element_type=F32)
                a = at if a is None else a + at
            m = functools.reduce(jnp.maximum, logits)
            ps = [jnp.exp2(lg - m) for lg in logits]
            rl = _rcp(functools.reduce(jnp.add, ps))
            ps = [p * rl for p in ps]
            cols = []
            for t in range(8):
                cs = slice(t * 128, (t + 1) * 128)
                acc = None
                for w in range(W):
                    o = PAD - DIL * w
                    tt = ps[w] * vw[o:o + RS, cs]
                    acc = tt if acc is None else acc + tt
                cols.append(acc)
            outs.append(_swap_lane_tiles(_pk(jnp.concatenate(cols, axis=1))))
        ob = _up(jnp.concatenate(outs, axis=0))
        b = jnp.dot(ob, _up(wob_u[...]), preferred_element_type=F32)
        g = jax.nn.sigmoid(jnp.sum(xb.astype(F32) * gw, axis=1, keepdims=True))
        res = g * a + (1.0 - g) * b

        @pl.when(r >= 2)
        def _():
            out_cp(r - 2, slot).wait()

        outs_v[slot] = res.astype(BF16)
        out_cp(r, slot).start()
        return carry

    jax.lax.fori_loop(0, nrf, fin_body, 0)
    out_cp(nrf - 2, (nrf - 2) % 2).wait()
    out_cp(nrf - 1, (nrf - 1) % 2).wait()


@jax.jit
def pallas_gated_mix__compressed_kv_cla__sliding_local_dilated__prompt_kernel(
    A_x, A_c_kv, A_w_q, A_w_uk, A_w_uv, A_w_o, B_x, B_wqkv, B_wo, gate_w):
    x = A_x.reshape(S, M)
    c = A_c_kv.reshape(S, DC)
    wq = A_w_q.reshape(M * H, D)
    wuk = A_w_uk.reshape(DC * H, D)
    wuv = A_w_uv.reshape(DC * H, D)
    wo = A_w_o.reshape(H * D, M)
    anyspec = pl.BlockSpec(memory_space=pl.ANY)
    out = pl.pallas_call(
        _kernel,
        grid=(1,),
        in_specs=[anyspec] * 8 + [pl.BlockSpec((M,), lambda i: (0,))],
        out_specs=anyspec,
        out_shape=jax.ShapeDtypeStruct((S, M), BF16),
        scratch_shapes=[
            pltpu.VMEM((S // 2, M), U32), pltpu.VMEM((S // 2, DC), U32),
            pltpu.VMEM((H, M // 2, D), U32), pltpu.VMEM((H, DC // 2, D), U32), pltpu.VMEM((H, DC // 2, D), U32),
            pltpu.VMEM((H * D // 2, M), U32), pltpu.VMEM((M // 2, DB), U32), pltpu.VMEM((M // 2, DB), U32), pltpu.VMEM((M // 2, DB), U32),
            pltpu.VMEM((DB // 2, DB), U32),
            pltpu.VMEM((S // 2, H * D), U32),
            pltpu.VMEM((S // 2, D), U32), pltpu.VMEM((S // 2, D), U32), pltpu.VMEM((S // 2, D), U32),
            pltpu.VMEM((2, S + PAD, DB), F32),
            pltpu.VMEM((NSLOT, M * H // NT1, D), BF16), pltpu.VMEM((NSLOT, DC * H // NT1, D), BF16),
            pltpu.VMEM((NSLOT, DC * H // NT1, D), BF16),
            pltpu.VMEM((NSLOT, RB, M), BF16), pltpu.VMEM((NSLOT, S // NT1, DC), BF16),
            pltpu.VMEM((M, DB), BF16), pltpu.VMEM((S // RB, M // (S // RB), DB), BF16),
            pltpu.VMEM((2, D, M), BF16), pltpu.VMEM((2, 32, DB), BF16), pltpu.VMEM((2, 32, DB), BF16),
            pltpu.VMEM((2, RF, M), BF16),
            pltpu.SemaphoreType.DMA((5, NSLOT)), pltpu.SemaphoreType.DMA((NKC,)),
            pltpu.SemaphoreType.DMA((S // RB,)), pltpu.SemaphoreType.DMA((3, 2)), pltpu.SemaphoreType.DMA((2,)),
        ],
        compiler_params=pltpu.CompilerParams(
            dimension_semantics=("arbitrary",), vmem_limit_bytes=110 * 1024 * 1024),
    )(x, c, wq, wuk, wuv, wo, B_wqkv, B_wo, gate_w)
    return out.reshape(1, S, M)
```

```python
import functools
import jax
import jax.numpy as jnp
import jax.experimental.pallas as pl
import jax.experimental.pallas.tpu as pltpu

S = 2048
M = 1024
H = 32
D = 128
DC = 512
DB = 1024
W = 8
DIL = 2
RF = 256
RB = 256
PAD = 16
NT1 = 16
NSLOT = 3
F32 = jnp.float32
BF16 = jnp.bfloat16
U32 = jnp.uint32
LOG2E = 1.4426950408889634
NEG = -1e9 * LOG2E
NT = (((1,), (1,)), ((), ()))
BLOCKS = [(1536, 512), (1024, 512), (512, 512), (0, 512)]
RPAD = 128
NKC = 8
FINSPLIT = 2
KCH = 512


def _pk(v):
    return pltpu.bitcast(v.astype(BF16), U32)


def _up(u):
    return pltpu.bitcast(u, BF16)


def _rcp(l):
    r = pl.reciprocal(l, approx=True)
    return r * (2.0 - l * r)


def _swap_lane_tiles(u):
    lane = jax.lax.broadcasted_iota(jnp.int32, (u.shape[0], 128), 1)
    t = [u[:, i * 128:(i + 1) * 128] for i in range(8)]
    for b in range(3):
        s = 4 << b
        lo = (lane & s) == 0
        n = list(t)
        for i in range(8):
            if not (i >> b) & 1:
                A, B = t[i], t[i | (1 << b)]
                n[i] = jnp.where(lo, A, pltpu.roll(B, s, 1))
                n[i | (1 << b)] = jnp.where(lo, pltpu.roll(A, 128 - s, 1), B)
        t = n
    return jnp.concatenate(t, axis=1)


def _kernel(x_hbm, c_hbm, wq_hbm, wuk_hbm, wuv_hbm, wo_hbm, wqkv_hbm, wob_hbm, gate_ref,
            out_hbm,
            xu, cu, wq_u, wuk_u, wuv_u, wo_u, wqb_u, wk_u, wv_u, wob_u, ctx_u, q_u, k_u, v_u,
            kvb_v, rq_v, ruk_v, ruv_v, rx_v, rc_v, rk_v, rv_v, jo_v, jq_v, jb_v, outs_v,
            rsem, wsem, vsem, jsem, osems):
    nrb = S // RB
    RQ = M * H // NT1
    RU = DC * H // NT1
    RC = S // NT1

    def x_cp(r, slot):
        return pltpu.make_async_copy(x_hbm.at[pl.ds(pl.multiple_of(r * RB, RB), RB), :], rx_v.at[slot], rsem.at[4, slot])

    def raw_cps(t, slot):
        return [
            pltpu.make_async_copy(wq_hbm.at[pl.ds(pl.multiple_of(t * RQ, RQ), RQ), :], rq_v.at[slot, pl.ds(0, RQ), :], rsem.at[0, slot]),
            pltpu.make_async_copy(wuk_hbm.at[pl.ds(pl.multiple_of(t * RU, RU), RU), :], ruk_v.at[slot, pl.ds(0, RU), :], rsem.at[1, slot]),
            pltpu.make_async_copy(wuv_hbm.at[pl.ds(pl.multiple_of(t * RU, RU), RU), :], ruv_v.at[slot, pl.ds(0, RU), :], rsem.at[2, slot]),
            pltpu.make_async_copy(c_hbm.at[pl.ds(pl.multiple_of(t * RC, RC), RC), :], rc_v.at[slot], rsem.at[3, slot]),
        ]

    def job_cps(h, slot):
        return [
            pltpu.make_async_copy(wo_hbm.at[pl.ds(pl.multiple_of(h * D, D), D), :], jo_v.at[slot], jsem.at[0, slot]),
            pltpu.make_async_copy(wqkv_hbm.at[pl.ds(pl.multiple_of(h * 32, 32), 32), pl.ds(0, DB)], jq_v.at[slot], jsem.at[1, slot]),
            pltpu.make_async_copy(wob_hbm.at[pl.ds(pl.multiple_of(h * 32, 32), 32), :], jb_v.at[slot], jsem.at[2, slot]),
        ]

    KR = M // NKC

    def wk_cp(i):
        return pltpu.make_async_copy(wqkv_hbm.at[pl.ds(i * KR, KR), pl.ds(DB, DB)], rk_v.at[pl.ds(i * KR, KR), :], wsem.at[i])

    VR = M // nrb

    def wv_cp(t):
        return pltpu.make_async_copy(wqkv_hbm.at[pl.ds(pl.multiple_of(t * VR, VR), VR), pl.ds(2 * DB, DB)],
                                     rv_v.at[t], vsem.at[t])

    for i in range(NKC):
        wk_cp(i).start()
    x_cp(0, 0).start()
    for c in raw_cps(0, 0):
        c.start()
    wv_cp(0).start()
    x_cp(1, 1).start()
    wv_cp(1).start()
    for c in raw_cps(1, 1):
        c.start()

    kvb_v[0, 0:PAD, :] = jnp.zeros((PAD, DB), F32)
    kvb_v[1, 0:PAD, :] = jnp.zeros((PAD, DB), F32)
    for i in range(NKC):
        wk_cp(i).wait()
        wk_u[i * KR // 2:(i + 1) * KR // 2, :] = _swap_lane_tiles(_pk(rk_v[i * KR:(i + 1) * KR, :]))

    rq_u = rq_v.bitcast(U32)
    ruk_u = ruk_v.bitcast(U32)
    ruv_u = ruv_v.bitcast(U32)

    def relayout(src_u, slot, dst, row0, nrows):
        for j in range(H // 2):
            u = src_u[slot, pl.ds(j, nrows, stride=H // 2), :]
            lo = pltpu.bitcast(u << 16, F32)
            hi = pltpu.bitcast(u & jnp.uint32(0xFFFF0000), F32)
            dst[2 * j, pl.ds(row0, nrows // 2), :] = _pk(lo)
            dst[2 * j + 1, pl.ds(row0, nrows // 2), :] = _pk(hi)

    def p1_body(mat, r, carry):
        t = mat * nrb + r
        slot = t % NSLOT

        @pl.when(t + 2 < NT1)
        def _():
            for c in raw_cps(t + 2, (t + 2) % NSLOT):
                c.start()

        if mat == 0:
            @pl.when(r + 2 < nrb)
            def _():
                x_cp(r + 2, (r + 2) % NSLOT).start()
                wv_cp(r + 2).start()

            x_cp(r, slot).wait()
            wv_cp(r).wait()
        else:
            @pl.when(r == nrb - 2)
            def _():
                for c in job_cps(0, 0):
                    c.start()

        for c in raw_cps(t, slot):
            c.wait()
        r0 = pl.multiple_of(r * RB, RB)
        hx = pl.multiple_of(r * (RB // 2), RB // 2)
        hq = pl.multiple_of(t * (M // NT1 // 2), M // NT1 // 2)
        hu = pl.multiple_of(t * (DC // NT1 // 2), DC // NT1 // 2)
        xb = rx_v[slot] if mat == 0 else _up(xu[pl.ds(hx, RB // 2), :])
        w_u = wk_u if mat == 0 else wv_u

        kvb_v[mat, pl.ds(r0 + PAD, RB), :] = jnp.dot(xb, _up(w_u[...]), preferred_element_type=F32)
        relayout(rq_u, slot, wq_u, hq, M // NT1)
        relayout(ruk_u, slot, wuk_u, hu, DC // NT1)
        relayout(ruv_u, slot, wuv_u, hu, DC // NT1)
        cu[pl.ds(pl.multiple_of(t * (RC // 2), RC // 2), RC // 2), :] = _pk(rc_v[slot])
        if mat == 0:
            wv_u[pl.ds(pl.multiple_of(r * (VR // 2), VR // 2), VR // 2), :] = _swap_lane_tiles(_pk(rv_v[r]))
            xu[pl.ds(hx, RB // 2), :] = _pk(xb)
        return carry

    jax.lax.fori_loop(0, nrb, functools.partial(p1_body, 0), 0)
    jax.lax.fori_loop(0, nrb, functools.partial(p1_body, 1), 0)

    qscale = (D ** -0.5) * LOG2E

    def head_body(h, carry):
        js = h % 2

        @pl.when(h + 1 < H)
        def _():
            for c in job_cps(h + 1, 1 - js):
                c.start()

        for c in job_cps(h, js):
            c.wait()
        q = jnp.dot(_up(xu[...]), _up(wq_u[h]), preferred_element_type=F32)
        q_u[...] = _pk(q * qscale)
        cb = _up(cu[...])
        k_u[...] = _pk(jnp.dot(cb, _up(wuk_u[h]), preferred_element_type=F32))
        v_u[...] = _pk(jnp.dot(cb, _up(wuv_u[h]), preferred_element_type=F32))
        wo_u[pl.ds(pl.multiple_of(h * (D // 2), D // 2), D // 2), :] = _pk(jo_v[js])
        wqb_u[pl.ds(pl.multiple_of(h * 16, 16), 16), :] = _swap_lane_tiles(_pk(jq_v[js]))
        wob_u[pl.ds(pl.multiple_of(h * 16, 16), 16), :] = _pk(jb_v[js])
        lane0 = pl.multiple_of(h * D, D)
        tri = (jax.lax.broadcasted_iota(jnp.int32, (128, 128), 1)
               <= jax.lax.broadcasted_iota(jnp.int32, (128, 128), 0))
        for r0, BQ in BLOCKS:
            G = BQ // 128
            qb = _up(q_u[r0 // 2:(r0 + BQ) // 2, :])
            mt = None
            if r0 > 0:
                sf = jax.lax.dot_general(qb, _up(k_u[0:r0 // 2, :]), NT, preferred_element_type=F32)
                mt = functools.reduce(jnp.maximum, [sf[:, t * 128:(t + 1) * 128] for t in range(r0 // 128)])
            sd = []
            for j in range(G):
                kj = _up(k_u[(r0 + j * 128) // 2:(r0 + (j + 1) * 128) // 2, :])
                sj = jax.lax.dot_general(qb[j * 128:], kj, NT, preferred_element_type=F32)
                top = jnp.where(tri, sj[:128], NEG)
                sd.append(top if j == G - 1 else jnp.concatenate([top, sj[128:]], axis=0))
            mg = []
            for i in range(G):
                ts = [sd[j][(i - j) * 128:(i - j + 1) * 128] for j in range(i + 1)]
                if mt is not None:
                    ts.append(mt[i * 128:(i + 1) * 128])
                mg.append(functools.reduce(jnp.maximum, ts))
            m = jnp.max(jnp.concatenate(mg, axis=0), axis=1, keepdims=True)
            run = [None] * G
            lrun = [None] * G
            if r0 > 0:
                pf = jnp.exp2(sf - m)
                lt = functools.reduce(jnp.add, [pf[:, t * 128:(t + 1) * 128] for t in range(r0 // 128)])
                acc = jnp.dot(pf.astype(BF16), _up(v_u[0:r0 // 2, :]), preferred_element_type=F32)
                run = [acc[i * 128:(i + 1) * 128] for i in range(G)]
                lrun = [lt[i * 128:(i + 1) * 128] for i in range(G)]
            for j in range(G):
                pj = jnp.exp2(sd[j] - m[j * 128:])
                aj = jnp.dot(pj.astype(BF16), _up(v_u[(r0 + j * 128) // 2:(r0 + (j + 1) * 128) // 2, :]),
                             preferred_element_type=F32)
                for i in range(j, G):
                    pa, pp = aj[(i - j) * 128:(i - j + 1) * 128], pj[(i - j) * 128:(i - j + 1) * 128]
                    run[i] = pa if run[i] is None else run[i] + pa
                    lrun[i] = pp if lrun[i] is None else lrun[i] + pp
                rl = _rcp(jnp.sum(lrun[j], axis=1, keepdims=True))
                ctx_u[(r0 + j * 128) // 2:(r0 + (j + 1) * 128) // 2, pl.ds(lane0, D)] = _pk(run[j] * rl)
        return carry

    jax.lax.fori_loop(0, H, head_body, 0)

    gw = gate_ref[...].astype(F32)[None, :]
    bscale = (32 ** -0.5) * LOG2E

    nrf = S // RF

    def out_cp(r, slot):
        r0 = pl.multiple_of(r * RF, RF)
        return pltpu.make_async_copy(outs_v.at[slot], out_hbm.at[pl.ds(r0, RF), :], osems.at[slot])

    def fin_body(r, carry):
        r0 = pl.multiple_of(r * RF, RF)
        hr = pl.multiple_of(r * (RF // 2), RF // 2)
        slot = r % 2
        xb = _up(xu[pl.ds(hr, RF // 2), :])
        qb = jnp.dot(xb, _up(wqb_u[...]), preferred_element_type=F32) * bscale
        NS = FINSPLIT
        RS = RF // NS
        lane = jax.lax.broadcasted_iota(jnp.int32, (RS, 128), 1)
        odd1 = (lane & 1) == 1
        odd2 = (lane & 2) == 2
        a = None
        outs = []
        for sc in range(NS):
            s0 = sc * RS
            kw = kvb_v[0, pl.ds(r0 + s0, RS + PAD), :]
            vw = kvb_v[1, pl.ds(r0 + s0, RS + PAD), :]
            logits = []
            for w in range(W):
                o = PAD - DIL * w
                pr = qb[s0:s0 + RS] * kw[o:o + RS]
                lg = functools.reduce(jnp.add, [pr[:, t * 128:(t + 1) * 128] for t in range(8)])
                lg = lg + jnp.where(odd1, pltpu.roll(lg, 1, 1), pltpu.roll(lg, 127, 1))
                lg = lg + jnp.where(odd2, pltpu.roll(lg, 2, 1), pltpu.roll(lg, 126, 1))
                if w > 0 and s0 < PAD:
                    row = r0 + jax.lax.broadcasted_iota(jnp.int32, (PAD, 128), 0)
                    top = jnp.where(row >= DIL * w, lg[:PAD], NEG)
                    lg = top if RS == PAD else jnp.concatenate([top, lg[PAD:]], axis=0)
                logits.append(lg)
            for kc in range(sc * (H * D // KCH) // NS, (sc + 1) * (H * D // KCH) // NS):
                ks = slice(kc * KCH, (kc + 1) * KCH)
                hs = slice(kc * KCH // 2, (kc + 1) * KCH // 2)
                at = jnp.dot(_up(ctx_u[pl.ds(hr, RF // 2), ks]), _up(wo_u[hs, :]), preferred_element_type=F32)
                a = at if a is None else a + at
            m = functools.reduce(jnp.maximum, logits)
            ps = [jnp.exp2(lg - m) for lg in logits]
            rl = _rcp(functools.reduce(jnp.add, ps))
            ps = [p * rl for p in ps]
            cols = []
            for t in range(8):
                cs = slice(t * 128, (t + 1) * 128)
                acc = None
                for w in range(W):
                    o = PAD - DIL * w
                    tt = ps[w] * vw[o:o + RS, cs]
                    acc = tt if acc is None else acc + tt
                cols.append(acc)
            outs.append(_swap_lane_tiles(_pk(jnp.concatenate(cols, axis=1))))
        ob = _up(jnp.concatenate(outs, axis=0))
        b = jnp.dot(ob, _up(wob_u[...]), preferred_element_type=F32)
        g = jax.nn.sigmoid(jnp.sum(xb.astype(F32) * gw, axis=1, keepdims=True))
        res = g * a + (1.0 - g) * b

        @pl.when(r >= 2)
        def _():
            out_cp(r - 2, slot).wait()

        outs_v[slot] = res.astype(BF16)
        out_cp(r, slot).start()
        return carry

    jax.lax.fori_loop(0, nrf, fin_body, 0)
    out_cp(nrf - 2, (nrf - 2) % 2).wait()
    out_cp(nrf - 1, (nrf - 1) % 2).wait()


@jax.jit
def pallas_gated_mix__compressed_kv_cla__sliding_local_dilated__prompt_kernel(
    A_x, A_c_kv, A_w_q, A_w_uk, A_w_uv, A_w_o, B_x, B_wqkv, B_wo, gate_w):
    x = A_x.reshape(S, M)
    c = A_c_kv.reshape(S, DC)
    wq = A_w_q.reshape(M * H, D)
    wuk = A_w_uk.reshape(DC * H, D)
    wuv = A_w_uv.reshape(DC * H, D)
    wo = A_w_o.reshape(H * D, M)
    anyspec = pl.BlockSpec(memory_space=pl.ANY)
    out = pl.pallas_call(
        _kernel,
        grid=(1,),
        in_specs=[anyspec] * 8 + [pl.BlockSpec((M,), lambda i: (0,))],
        out_specs=anyspec,
        out_shape=jax.ShapeDtypeStruct((S, M), BF16),
        scratch_shapes=[
            pltpu.VMEM((S // 2, M), U32), pltpu.VMEM((S // 2, DC), U32),
            pltpu.VMEM((H, M // 2, D), U32), pltpu.VMEM((H, DC // 2, D), U32), pltpu.VMEM((H, DC // 2, D), U32),
            pltpu.VMEM((H * D // 2, M), U32), pltpu.VMEM((M // 2, DB), U32), pltpu.VMEM((M // 2, DB), U32), pltpu.VMEM((M // 2, DB), U32),
            pltpu.VMEM((DB // 2, DB), U32),
            pltpu.VMEM((S // 2, H * D), U32),
            pltpu.VMEM((S // 2, D), U32), pltpu.VMEM((S // 2, D), U32), pltpu.VMEM((S // 2, D), U32),
            pltpu.VMEM((2, S + PAD, DB), F32),
            pltpu.VMEM((NSLOT, M * H // NT1 + RPAD, D), BF16), pltpu.VMEM((NSLOT, DC * H // NT1 + RPAD, D), BF16),
            pltpu.VMEM((NSLOT, DC * H // NT1 + RPAD, D), BF16),
            pltpu.VMEM((NSLOT, RB, M), BF16), pltpu.VMEM((NSLOT, S // NT1, DC), BF16),
            pltpu.VMEM((M, DB), BF16), pltpu.VMEM((S // RB, M // (S // RB), DB), BF16),
            pltpu.VMEM((2, D, M), BF16), pltpu.VMEM((2, 32, DB), BF16), pltpu.VMEM((2, 32, DB), BF16),
            pltpu.VMEM((2, RF, M), BF16),
            pltpu.SemaphoreType.DMA((5, NSLOT)), pltpu.SemaphoreType.DMA((NKC,)),
            pltpu.SemaphoreType.DMA((S // RB,)), pltpu.SemaphoreType.DMA((3, 2)), pltpu.SemaphoreType.DMA((2,)),
        ],
        compiler_params=pltpu.CompilerParams(
            dimension_semantics=("arbitrary",), vmem_limit_bytes=110 * 1024 * 1024),
    )(x, c, wq, wuk, wuv, wo, B_wqkv, B_wo, gate_w)
    return out.reshape(1, S, M)
```
